```python
import os as _os
_os.environ.setdefault("JAX_PLATFORMS", "cpu")
import jax
import jax.numpy as jnp

def _softmax(x, axis=-1):
    return jax.nn.softmax(x, axis=axis)
def _gelu(x):
    return jax.nn.gelu(x, approximate=True)
def _silu(x):
    return jax.nn.silu(x)
def _sigmoid(x):
    return jax.nn.sigmoid(x)
def _layernorm(x, axis=-1, eps=1e-5):
    m = jnp.mean(x, axis=axis, keepdims=True)
    v = jnp.var(x, axis=axis, keepdims=True)
    return (x - m) / jnp.sqrt(v + eps)
def _scatter_add(tgt, idx, src, axis=0):
    return tgt.at[idx].add(src)
def _segment_sum(src, seg, n):
    return jax.ops.segment_sum(src, seg, n)
class _Rng:
    def __init__(self, key):
        self._k = key
    def _next(self):
        self._k, sub = jax.random.split(self._k)
        return sub
    def normal(self, shape):
        return jax.random.normal(self._next(), shape, dtype=jnp.bfloat16)
    def randint(self, lo, hi, shape):
        return jax.random.randint(self._next(), shape, lo, hi, dtype=jnp.int32)
    def uniform(self, shape, lo=0.0, hi=1.0):
        return jax.random.uniform(self._next(), shape, jnp.bfloat16, lo, hi)
    def permutation(self, n):
        return jax.random.permutation(self._next(), n)


kernel_name = 'sequential_preLN__sliding_block__dense_activation_gelu__prompt'

def setup_inputs():
    _rng = _Rng(jax.random.key(int.from_bytes(__import__("os").urandom(4), "little")))
    _w = (lambda a: (lambda t: t.astype(jnp.bfloat16) if jnp.issubdtype(t.dtype, jnp.floating) else t)(jnp.asarray(a)))
    def _A_setup():
        B, S, D = 1, 2048, 640
        return {
            "x": _w((lambda *s: _rng.normal(s) * 0.05)(B, S, D)),
            "wqkv": _w((lambda *s: _rng.normal(s) * 0.05)(D, 3 * D)),
            "wo": _w((lambda *s: _rng.normal(s) * 0.05)(D, D)),
        }
    _A_in = _A_setup()

    def _B_setup():
        B, S, D, F = 1, 2048, 640, 1536
        return {
            "x": _w((lambda *s: _rng.normal(s) * 0.05)(B, S, D)),
            "w1": _w((lambda *s: _rng.normal(s) * 0.8)(D, F) * (D ** -0.5)),
            "b1": _w((lambda *s: _rng.normal(s) * 0.8)(F) * 0.01),
            "w2": _w((lambda *s: _rng.normal(s) * 0.8)(F, D) * (F ** -0.5)),
            "b2": _w((lambda *s: _rng.normal(s) * 0.05)(D) * 0.01),
        }
    _B_in = _B_setup()

    return {
        "A_x": _A_in["x"],
        "A_wqkv": _A_in["wqkv"],
        "A_wo": _A_in["wo"],
        "B_x": _B_in["x"],
        "B_w1": _B_in["w1"],
        "B_b1": _B_in["b1"],
        "B_w2": _B_in["w2"],
        "B_b2": _B_in["b2"],
    }

def reference(A_x, A_wqkv, A_wo, B_x, B_w1, B_b1, B_w2, B_b2):
    def _A_ref(x, wqkv, wo):
        B, S, D = x.shape
        H = 32; Dh = D // H; W = 256
        qkv = (lambda x, *d: x.transpose(*d))((x @ wqkv).reshape(B, S, 3, H, Dh), 2, 0, 3, 1, 4)
        q, k, v = qkv[0], qkv[1], qkv[2]
        scores = jnp.einsum("bhqd,bhkd->bhqk", q, k) * (Dh ** -0.5)
        idx = jnp.arange(S)
        mask = (idx[:, None] - idx[None, :] >= 0) & (idx[:, None] - idx[None, :] < W)
        scores = jnp.where(mask[None, None], scores, -1e9)
        p = _softmax(scores, axis=-1)
        o = jnp.einsum("bhqk,bhkd->bhqd", p, v)
        return (lambda x, *d: x.transpose(*d))(o, 0, 2, 1, 3).reshape(B, S, D) @ wo

    def _B_ref(x, w1, b1, w2, b2):
        h = jnp.einsum("bsd,df->bsf", x, w1) + b1
        h = _gelu(h)
        return jnp.einsum("bsf,fd->bsd", h, w2) + b2

    x = A_x
    h = x + _A_ref(_layernorm(x, axis=-1), A_wqkv, A_wo)
    h2 = h + _B_ref(_layernorm(h, axis=-1), B_w1, B_b1, B_w2, B_b2)
    return h2
```

```python
import functools
import math

import jax
import jax.numpy as jnp
from jax import lax
import jax.experimental.pallas as pl
import jax.experimental.pallas.tpu as pltpu

S = 2048
D = 640
F = 1536
H = 32
DH = 20
W = 256
NG = 8
EPS = 1e-5
QSCALE = (DH ** -0.5) * math.log2(math.e)
ONE_WORD = 0x3F803F80

f32 = jnp.float32
bf16 = jnp.bfloat16
i32 = jnp.int32


def _ln(x):
    m = jnp.mean(x, axis=-1, keepdims=True)
    xc = x - m
    v = jnp.mean(xc * xc, axis=-1, keepdims=True)
    return xc * lax.rsqrt(v + EPS)


def _gelu(x):
    c = math.sqrt(2.0 / math.pi)
    return 0.5 * x * (1.0 + jnp.tanh(c * (x + 0.044715 * (x * x * x))))


def _pack_i(a):
    R, C = a.shape
    a3 = a.reshape(R // 16, 16, C)
    w = pltpu.pack_elementwise([a3[:, 0:8, :], a3[:, 8:16, :]], packed_dtype=bf16)
    return w.reshape(R // 2, C)


def _group_tile(a, g, lane, zero_rest):
    lo = 80 * g
    t, off = lo // 128, lo % 128
    lo_t = a[:, 128 * t:128 * t + 128]
    if off + 80 <= 128:
        if zero_rest:
            return jnp.where((lane >= off) & (lane < off + 80), lo_t, 0.0)
        return lo_t
    e = off + 80 - 128
    hi_t = a[:, 128 * (t + 1):128 * (t + 2)]
    if zero_rest:
        return jnp.where(lane < e, hi_t, jnp.where(lane >= off, lo_t, 0.0))
    return jnp.where(lane < e, hi_t, lo_t)


def _sel(m, t, f_):
    if t is None and f_ is None:
        return None
    if t is None:
        t = 0
    if f_ is None:
        f_ = 0
    return jnp.where(m, t, f_)


def _kernel(x_ref, wqkv_ref, wo_ref, w1_ref, b1_ref, w2_ref, b2_ref, o_ref,
            kg_ref, vt_ref, wvt_ref, *, TQ, DEPTH):
    i = pl.program_id(0)
    NB = TQ // 128

    @pl.when(i == 0)
    def _init():
        lane1 = lax.broadcasted_iota(i32, (W // 2, 128), 1)
        for g in range(NG):
            sp = (80 * g + 80) % 128
            kg_ref[g, 0:W // 2, :] = jnp.where(lane1 == sp, ONE_WORD, 0).astype(i32)
        vt_ref[0:2] = jnp.zeros((2, H * 16, 128), i32)
        wvt_ref[...] = wqkv_ref[:, 2 * D:3 * D].astype(f32).T.astype(bf16)

    x = x_ref[...].astype(f32)
    xnf = _ln(x)
    xn = xnf.astype(bf16)
    xs_ = pltpu.bitcast(_pack_i(xnf), bf16)
    qk = jnp.dot(xn, wqkv_ref[:, 0:2 * D], preferred_element_type=f32)
    vt = lax.dot_general(wvt_ref[...], xs_, (((1,), (1,)), ((), ())),
                         preferred_element_type=f32)
    q = qk[:, 0:D] * QSCALE
    k = qk[:, D:2 * D]

    laneq = lax.broadcasted_iota(i32, (TQ, 128), 1)
    row0 = pl.multiple_of(i * (TQ // 2), TQ // 2)
    qg = []
    for g in range(NG):
        kg_ref[g, pl.ds(row0 + W // 2, TQ // 2), :] = pltpu.bitcast(
            _group_tile(k, g, laneq, True).astype(bf16), i32)
        qg.append(_group_tile(q, g, laneq, False))

    vtw = pltpu.bitcast(vt.astype(bf16), i32)
    sub8 = lax.broadcasted_iota(i32, (8, TQ), 0)
    pieces = []
    for h in range(H):
        g, hh = h // 4, h % 4
        w0 = 40 * g + 8 * hh
        a = vtw[w0:w0 + 8]
        b = vtw[w0 + 8:w0 + 16]
        if hh < 2:
            b = jnp.where(sub8 >= 4, ONE_WORD, b)
        else:
            a = jnp.where(sub8 < 4, ONE_WORD, a)
        pieces += [a, b]
    vtp = jnp.concatenate(pieces, axis=0)
    for nb in range(NB):
        vt_ref[i * NB + nb + 2] = vtp[:, 128 * nb:128 * nb + 128]

    lane16 = lax.broadcasted_iota(i32, (16, 128), 1)
    lane32 = lax.broadcasted_iota(i32, (32, 128), 1)
    r32 = lax.broadcasted_iota(i32, (32, 128), 0)
    tri = r32 > (lane32 & 31)
    rw = lax.broadcasted_iota(i32, (16, 128), 0)
    rw = (rw & 7) + 2 * (rw & 8)
    cw = lane16 & 31
    m_old = (jnp.where(rw > cw, 0xFFFF, 0) | jnp.where(rw + 8 > cw, -65536, 0)).astype(i32)
    m_new = ~m_old
    s_odd = (lane16 & 32) != 0
    s_hi = (lane16 & 64) != 0
    sub8b = lax.broadcasted_iota(i32, (8, 128), 0) < 4

    def qk_stage(nb, g):
        off = (80 * g) % 128
        rel = (lane32 - off) & 127
        cneg = jnp.where(rel == 80, -2.0 ** 100, 0.0).astype(f32)
        hmask = [(rel >= 20 * hh) & (rel < 20 * hh + 20) for hh in range(4)]
        xs = []
        for j in range(4):
            jj = 4 * nb + j
            qs = qg[g][32 * jj:32 * jj + 32]
            bmat = jnp.concatenate(
                [jnp.where(hmask[s ^ j], qs, cneg) for s in range(4)], axis=0).astype(bf16)
            kwin = pltpu.bitcast(kg_ref[g, pl.ds(row0 + 16 * jj, 144), :], bf16)
            st = lax.dot_general(kwin, bmat, (((1,), (1,)), ((), ())),
                                 preferred_element_type=f32)
            edge = jnp.where(tri, st[0:32], st[256:288])
            sm = jnp.concatenate([st[32:256], edge], axis=0)
            mx = jnp.max(sm, axis=0, keepdims=True)
            pw = _pack_i(jnp.exp2(sm - mx))
            pe = pw[112:128]
            blk = [pe & m_old] + [pw[16 * b:16 * b + 16] for b in range(7)] + [pe & m_new]
            xs.append(blk)
        return xs

    def pv_stage(nb, g, xs):
        wrows = [[], [], [], []]
        for a in range(12):
            X = [xs[j][a - j] if 0 <= a - j <= 8 else None for j in range(4)]
            Y = [_sel(s_odd, X[1], X[0]), _sel(s_odd, X[0], X[1]),
                 _sel(s_odd, X[3], X[2]), _sel(s_odd, X[2], X[3])]
            Z = [_sel(s_hi, Y[2], Y[0]), _sel(s_hi, Y[3], Y[1]),
                 _sel(s_hi, Y[0], Y[2]), _sel(s_hi, Y[1], Y[3])]
            for hh in range(4):
                wrows[hh].append(Z[hh])
        on = []
        kb = i * NB + nb
        for hh in range(4):
            h = 4 * g + hh
            wm = pltpu.bitcast(jnp.concatenate(wrows[hh], axis=0), bf16)
            vl = pltpu.bitcast(jnp.concatenate(
                [vt_ref[kb + t, 16 * h:16 * h + 16, :] for t in range(3)], axis=1), bf16)
            ot = jnp.dot(vl, wm, preferred_element_type=f32)
            den = ot[24:32] if hh < 2 else ot[0:8]
            r = 1.0 / den
            on.append([ot[8 * t:8 * t + 8] * r for t in range(4)])
        return [on[0][0], on[0][1], jnp.where(sub8b, on[0][2], on[1][0]),
                on[1][1], on[1][2], on[2][1], on[2][2],
                jnp.where(sub8b, on[2][3], on[3][1]), on[3][2], on[3][3]]

    def finish_block(ot_rows):
        otc = jnp.concatenate(ot_rows, axis=0)
        tw = pltpu.bitcast(otc.T.astype(bf16), i32)
        lane640 = lax.broadcasted_iota(i32, (16, D), 1)
        hid = lane640 // DH
        b0 = (hid & 1) != 0
        b1 = (hid & 2) != 0
        X = [tw[16 * j:16 * j + 16] for j in range(4)]
        Y = [jnp.where(b0, X[j ^ 1], X[j]) for j in range(4)]
        return [jnp.where(b1, Y[j ^ 2], Y[j]) for j in range(4)]

    items = [(nb, g) for nb in range(NB) for g in range(NG)]
    pend = {}
    o_blocks = []
    ot_rows = []
    for n in range(len(items) + DEPTH):
        if n < len(items):
            pend[n] = qk_stage(*items[n])
        m = n - DEPTH
        if m >= 0:
            ot_rows += pv_stage(*items[m], pend.pop(m))
            if items[m][1] == NG - 1:
                o_blocks += finish_block(ot_rows)
                ot_rows = []
    o = pltpu.bitcast(jnp.concatenate(o_blocks, axis=0), bf16)

    h1 = x + jnp.dot(o, wo_ref[...], preferred_element_type=f32)
    hn = _ln(h1).astype(bf16)
    u = jnp.dot(hn, w1_ref[...], preferred_element_type=f32) + b1_ref[...].astype(f32).reshape(1, F)
    gl = _gelu(u).astype(bf16)
    y = jnp.dot(gl, w2_ref[...], preferred_element_type=f32) + b2_ref[...].astype(f32).reshape(1, D)
    o_ref[...] = (h1 + y).astype(o_ref.dtype)


def make(TQ=256, DEPTH=1):
    @jax.jit
    def fn(A_x, A_wqkv, A_wo, B_x, B_w1, B_b1, B_w2, B_b2):
        del B_x
        const = lambda i: (0, 0)
        return pl.pallas_call(
            functools.partial(_kernel, TQ=TQ, DEPTH=DEPTH),
            grid=(S // TQ,),
            in_specs=[
                pl.BlockSpec((None, TQ, D), lambda i: (0, i, 0)),
                pl.BlockSpec((D, 3 * D), const),
                pl.BlockSpec((D, D), const),
                pl.BlockSpec((D, F), const),
                pl.BlockSpec((F,), lambda i: (0,)),
                pl.BlockSpec((F, D), const),
                pl.BlockSpec((D,), lambda i: (0,)),
            ],
            out_specs=pl.BlockSpec((None, TQ, D), lambda i: (0, i, 0)),
            out_shape=jax.ShapeDtypeStruct((1, S, D), bf16),
            scratch_shapes=[
                pltpu.VMEM((NG, (S + W) // 2, 128), i32),
                pltpu.VMEM((S // 128 + 2, H * 16, 128), i32),
                pltpu.VMEM((D, D), bf16),
            ],
            compiler_params=pltpu.CompilerParams(
                dimension_semantics=("arbitrary",),
                vmem_limit_bytes=100 * 2**20),
        )(A_x, A_wqkv, A_wo, B_w1, B_b1, B_w2, B_b2)
    return fn


pallas_sequential_preLN__sliding_block__dense_activation_gelu__prompt_kernel = make(TQ=256,DEPTH=2)
```

```python
import functools
import math

import jax
import jax.numpy as jnp
from jax import lax
import jax.experimental.pallas as pl
import jax.experimental.pallas.tpu as pltpu

S = 2048
D = 640
F = 1536
H = 32
DH = 20
W = 256
NG = 8
TQ = 256
NB = TQ // 128
NU = S // TQ
EPS = 1e-5
QSCALE = (DH ** -0.5) * math.log2(math.e)
NEG_WORD = -243207808
ONE_WORD = 0x3F803F80

f32 = jnp.float32
bf16 = jnp.bfloat16
i32 = jnp.int32

DEFAULT_CFG = dict(
    DEPTH=2,
    REL=((0, 0), (0, 96), (0, 200)),
    SS=16, SD=2,
    WOD=2,
    INS=('pv',),
    TAIL=(2, 2),
    START=1,
    VCH=4,
    ORDER='f1,f2a,k,v,f2b,q',
    BIAS=0.5,
    ONLY=None,
    NSPL=(1, 1, 1, 1, 1, 1),
    PLAN=('x0 k', 'q v x1', '1 2 o', '', 'x2', 'x3', 'x4 x5 x6 x7'),
    WOW=2,
    MERGEW=0,
    OSPL=4,
    first=dict(DEPTH=2, REL=(None, (0, 96), (0, 200)), SS=16, SD=2, WOD=3, INS=('pv', 'qk'),
               TAIL=(1, 1), START=3, VCH=4, ORDER='k,f1,f2a,v,f2b,q', BIAS=1.0),
    mid=dict(DEPTH=1, REL=((0, 0), (0, 96), (0, 144)), SS=16, SD=2, WOD=3, INS=('pv',),
             TAIL=(1, 4), START=1, VCH=4, ORDER='f1,f2a,f2b,k,v,q', BIAS=1.0),
    last=dict(DEPTH=1, REL=((0, 0), (0, 96), (0, 144)), SS=16, SD=2, WOD=3, INS=('pv',),
              TAIL=(1, 4), START=1, VCH=4, ORDER='f1,f2a,f2b,k,v,q', BIAS=1.0),
)


def _ln(x):
    m = jnp.mean(x, axis=-1, keepdims=True)
    xc = x - m
    v = jnp.mean(xc * xc, axis=-1, keepdims=True)
    return xc * lax.rsqrt(v + EPS)


def _gelu(x):
    c = math.sqrt(2.0 / math.pi)
    return 0.5 * x * (1.0 + jnp.tanh(c * (x + 0.044715 * (x * x * x))))


def _pack_i(a):
    R, C = a.shape
    a3 = a.reshape(R // 16, 16, C)
    w = pltpu.pack_elementwise([a3[:, 0:8, :], a3[:, 8:16, :]], packed_dtype=bf16)
    return w.reshape(R // 2, C)


def _words(a):
    return pltpu.bitcast(a.astype(bf16), i32)


def _as_bf16(w):
    return pltpu.bitcast(w, bf16)


def _group_tile(tiles, g, lane, zero_rest):
    lo = 80 * g
    t, off = lo // 128, lo % 128
    if off + 80 <= 128:
        if zero_rest:
            return jnp.where((lane >= off) & (lane < off + 80), tiles[t], 0)
        return tiles[t]
    e = off + 80 - 128
    if zero_rest:
        return jnp.where(lane < e, tiles[t + 1], jnp.where(lane >= off, tiles[t], 0))
    return jnp.where(lane < e, tiles[t + 1], tiles[t])


def _groups_ready(t):
    return [g for g in range(NG) if (80 * g + 79) // 128 == t]


def _sel(m, t, f_):
    if t is None and f_ is None:
        return None
    if t is None:
        t = 0
    if f_ is None:
        f_ = 0
    return jnp.where(m, t, f_)


class _Refs:
    pass


def _a_items(R, u, base, du, par, cfg, q_ref=None, free=False):
    st = {}
    xn_ref, xs_ref = R.xn[par], R.xs[par]
    q_ref = R.q if q_ref is None else q_ref
    row0 = base['krow'] + du * (TQ // 2)

    def ln1():
        x = R.x[pl.ds(base['xrow'] + du * TQ, TQ), :].astype(f32)
        xnf = _ln(x)
        xn_ref[...] = _words(xnf)
        xs_ref[...] = _pack_i(xnf)

    def kproj(t):
        k = jnp.dot(_as_bf16(xn_ref[...]), R.wk[:, 128 * t:128 * t + 128],
                    preferred_element_type=f32)
        st[('k', t)] = _words(k)
        lane = lax.broadcasted_iota(i32, (TQ // 2, 128), 1)
        tiles = {tt: st[('k', tt)] for tt in range(t + 1)}
        for g in _groups_ready(t):
            R.kg[g, pl.ds(row0 + W // 2, TQ // 2), :] = _group_tile(tiles, g, lane, True)

    def qproj(t):
        q = jnp.dot(_as_bf16(xn_ref[...]), R.wq[:, 128 * t:128 * t + 128],
                    preferred_element_type=f32) * QSCALE
        st[('q', t)] = _words(q)
        lane = lax.broadcasted_iota(i32, (TQ // 2, 128), 1)
        tiles = {tt: st[('q', tt)] for tt in range(t + 1)}
        for g in _groups_ready(t):
            q_ref[g] = _group_tile(tiles, g, lane, False)

    def vproj(c):
        gpc = NG // cfg['VCH']
        m0 = 80 * gpc * c
        vt = lax.dot_general(R.wvt[m0:m0 + 80 * gpc, :], _as_bf16(xs_ref[...]),
                             (((1,), (1,)), ((), ())), preferred_element_type=f32)
        vtw = _words(vt)
        sub8 = lax.broadcasted_iota(i32, (8, TQ), 0)
        pieces = []
        for gg in range(gpc):
            for hh in range(4):
                w0 = 40 * gg + 8 * hh
                a = vtw[w0:w0 + 8]
                b = vtw[w0 + 8:w0 + 16]
                if hh < 2:
                    b = jnp.where(sub8 >= 4, ONE_WORD, b)
                else:
                    a = jnp.where(sub8 < 4, ONE_WORD, a)
                pieces += [a, b]
        vtp = jnp.concatenate(pieces, axis=0)
        for nb in range(NB):
            R.vt[base['kb'] + du * NB + nb + 2, 64 * gpc * c:64 * gpc * (c + 1), :] = (
                vtp[:, 128 * nb:128 * nb + 128])

    return dict(
        ln=[('ln1', ln1, 0)],
        k=[('k', functools.partial(kproj, t), 320) for t in range(5)],
        q=[('q', functools.partial(qproj, t), 320, None if free else ('qk', NG + max(_groups_ready(t))), None)
           for t in range(5)],
        v=[('v', functools.partial(vproj, c), 1600 // cfg['VCH']) for c in range(cfg['VCH'])],
    )


def _b_items(R, base, du, par, cfg, z, q_ref=None, hbuf=0):
    st = {}
    s_ref, ot_ref = R.s, R.ot
    q_ref = R.q if q_ref is None else q_ref
    h1_ref, hn_ref = R.h1[hbuf], R.hn[hbuf]
    row0 = base['krow'] + du * (TQ // 2)
    DEPTH, SS, SD = cfg['DEPTH'], cfg['SS'], cfg['SD']

    lane16 = lax.broadcasted_iota(i32, (16, 128), 1)
    r16 = lax.broadcasted_iota(i32, (16, 128), 0)
    cw = lane16 & 31
    tri0 = r16 > cw
    tri1 = r16 + 16 > cw
    rw = (r16 & 7) + 2 * (r16 & 8)
    m_old = (jnp.where(rw > cw, 0xFFFF, 0) | jnp.where(rw + 8 > cw, -65536, 0)).astype(i32)
    m_new = ~m_old
    s_odd = (lane16 & 32) != 0
    s_hi = (lane16 & 64) != 0
    sub8b = lax.broadcasted_iota(i32, (8, 128), 0) < 4

    def qk_stage(n):
        nb, g = n // NG, n % NG
        off = (80 * g) % 128
        rel = (lane16 - off) & 127
        cneg = jnp.where(rel == 80, NEG_WORD, 0).astype(i32)
        hmask = [(rel >= 20 * hh) & (rel < 20 * hh + 20) for hh in range(4)]
        for j in range(4):
            jj = 4 * nb + j
            qs = q_ref[g, 16 * jj:16 * jj + 16, :]
            bmat = _as_bf16(jnp.concatenate(
                [jnp.where(hmask[s ^ j], qs, cneg) for s in range(4)], axis=0))
            kw = R.kg[g, pl.ds(row0 + 16 * jj, 144), :]
            kwin = _as_bf16(jnp.concatenate(
                [kw[16:128], kw[0:8], kw[128:136], kw[8:16], kw[136:144]], axis=0))
            s_t = lax.dot_general(kwin, bmat, (((1,), (1,)), ((), ())),
                                  preferred_element_type=f32)
            slot = n * 4 + j
            e0 = jnp.where(tri0, s_t[224:240], s_t[240:256])
            e1 = jnp.where(tri1, s_t[256:272], s_t[272:288])
            sm = jnp.concatenate([s_t[0:224], e0, e1], axis=0)
            m = None
            for r in range(0, 256, 8):
                v = sm[r:r + 8]
                if m is None:
                    m = v
                    s_ref[slot, r:r + 8, :] = v
                else:
                    m = jnp.maximum(m, v)
                    s_ref[slot, r:r + 8, :] = jnp.minimum(v, m)
            st[('mx', n, j)] = jnp.max(m, axis=0, keepdims=True)
            st[('st', n, j)] = s_t

    def sm_stage(n):
        for j in range(4):
            slot = n * 4 + j
            mx = jnp.broadcast_to(st.pop(('mx', n, j)), (8, 128))
            hist = []
            for r in range(0, 256, SS):
                if len(hist) >= SD:
                    mx = jnp.maximum(mx, hist[-SD] - 3e38)
                p = jnp.exp2(s_ref[slot, r:r + SS, :] - jnp.concatenate([mx] * (SS // 8), axis=0))
                hist.append(p[SS - 8:SS])
                R.p[n % 3][j, r // 2:(r + SS) // 2, :] = _pack_i(p)

    def pv_stage(n):
        nb, g = n // NG, n % NG
        p_ref = R.p[n % 3]
        kb = base['kb'] + du * NB + nb
        acc = [None] * 4
        for t in range(3):
            spec = cfg['REL'][t]
            if spec is not None and ('st', n + DEPTH, spec[0]) in st:
                s_t = st[('st', n + DEPTH, spec[0])]
                p_ref[4, 8 * t:8 * t + 8, :] = pltpu.bitcast(s_t[spec[1]:spec[1] + 8], i32)

            def blk(j, b):
                if b < 0 or b > 8:
                    return None
                if b == 0:
                    return p_ref[z + j, 112:128, :] & m_old
                if b == 8:
                    return p_ref[z + j, 112:128, :] & m_new
                return p_ref[z + j, 16 * (b - 1):16 * b, :]

            wrows = [[], [], [], []]
            for a in range(4 * t, 4 * t + 4):
                X = [blk(j, a - j) for j in range(4)]
                Y = [_sel(s_odd, X[1], X[0]), _sel(s_odd, X[0], X[1]),
                     _sel(s_odd, X[3], X[2]), _sel(s_odd, X[2], X[3])]
                Z = [_sel(s_hi, Y[2], Y[0]), _sel(s_hi, Y[3], Y[1]),
                     _sel(s_hi, Y[0], Y[2]), _sel(s_hi, Y[1], Y[3])]
                for hh in range(4):
                    wrows[hh].append(Z[hh])
            for hh in range(4):
                h = 4 * g + hh
                wm = _as_bf16(jnp.concatenate(wrows[hh], axis=0))
                vl = _as_bf16(R.vt[kb + t, 16 * h:16 * h + 16, :])
                ot = jnp.dot(vl, wm, preferred_element_type=f32)
                acc[hh] = ot if acc[hh] is None else acc[hh] + ot
        on = []
        for hh in range(4):
            ot = acc[hh]
            den = ot[24:32] if hh < 2 else ot[0:8]
            r = 1.0 / den
            on.append([ot[8 * t:8 * t + 8] * r for t in range(4)])
        ot_ref[nb, 80 * g:80 * g + 80, :] = jnp.concatenate(
            [on[0][0], on[0][1], jnp.where(sub8b, on[0][2], on[1][0]),
             on[1][1], on[1][2], on[2][1], on[2][2],
             jnp.where(sub8b, on[2][3], on[3][1]), on[3][2], on[3][3]], axis=0)

    def wo_stage(nb):
        t = ot_ref[nb].T
        lane640 = lax.broadcasted_iota(i32, (32, D), 1)
        hid = lane640 // DH
        b0 = (hid & 1) != 0
        b1 = (hid & 2) != 0
        X = [t[32 * j:32 * j + 32] for j in range(4)]
        Y = [jnp.where(b0, X[j ^ 1], X[j]) for j in range(4)]
        Z = [jnp.where(b1, Y[j ^ 2], Y[j]) for j in range(4)]
        o = jnp.concatenate(Z, axis=0).astype(bf16)
        x = R.x[pl.ds(base['xrow'] + du * TQ + 128 * nb, 128), :].astype(f32)
        h1 = x + jnp.dot(o, R.wo[...], preferred_element_type=f32)
        h1_ref[128 * nb:128 * nb + 128, :] = h1
        hn_ref[64 * nb:64 * nb + 64, :] = _words(_ln(h1))

    items = []
    NA = NB * NG
    pend = []
    for n in range(NA + DEPTH):
        if n < NA:
            items.append(('qk', functools.partial(qk_stage, n), 288, n))
            items.append(('sm', functools.partial(sm_stage, n), 0))
        m = n - DEPTH
        if m >= 0:
            items.append(('pv', functools.partial(pv_stage, m), 96))
            if pend and n >= pend[0][0]:
                items.append(pend.pop(0)[1])
            if m % NG == NG - 1:
                pend.append((n + cfg['WOD'], ('wo', functools.partial(wo_stage, m // NG), 800, m // NG)))
    items += [w[1] for w in pend]
    return items


def _c_items(R, base, du, par, hbuf=0, free=False):
    h1_ref, hn_ref, g_ref = R.h1[hbuf], R.hn[hbuf], R.g[par]
    w0, w1 = (None, None) if free else (('wo', 0), ('wo', 1))

    def f1(c):
        u = jnp.dot(_as_bf16(hn_ref[...]), R.w1[:, 128 * c:128 * c + 128],
                    preferred_element_type=f32)
        u = u + R.b1[128 * c:128 * c + 128].astype(f32).reshape(1, 128)
        g_ref[:, 128 * c:128 * c + 128] = _words(_gelu(u))

    def f2(m, n):
        g = _as_bf16(g_ref[64 * m:64 * m + 64, :])
        y = jnp.dot(g, R.w2[:, 128 * n:128 * n + 128], preferred_element_type=f32)
        y = y + R.b2[128 * n:128 * n + 128].astype(f32).reshape(1, 128)
        R.o[pl.ds(base['xrow'] + du * TQ + 128 * m, 128), 128 * n:128 * n + 128] = (
            h1_ref[128 * m:128 * m + 128, 128 * n:128 * n + 128] + y).astype(bf16)

    return dict(
        f1=[('f1', functools.partial(f1, c), 320, None, w0) for c in range(F // 128)],
        f2a=[('f2', functools.partial(f2, 0, n), 384, None, w0) for n in range(D // 128)],
        f2b=[('f2', functools.partial(f2, 1, n), 384, None, w1) for n in range(D // 128)],
    )


def _merge(main, fill, cfg):
    fill = [it if len(it) == 5 else it + (None, None) for it in fill]
    t1, t2 = cfg['TAIL']
    t2 = min(t2, len(fill))
    t1 = min(t1, len(fill) - t2)
    nmid = len(fill) - t1 - t2
    first = cfg['START']
    tot_f = sum(it[2] for it in main[first:-1])
    tot_b = sum(it[2] for it in fill[:nmid])
    out, done = [], set()
    todo = list(range(len(fill)))
    acc = [0, 0]

    def emit(k):
        todo.remove(k)
        out.append(fill[k])
        acc[1] += fill[k][2]

    for k, it in enumerate(main):
        tag = (it[0], it[3]) if len(it) > 3 else None
        if k == len(main) - 1:
            for f in [f for f in todo if f < nmid + t1]:
                emit(f)
        elif k >= first and it[0] in cfg['INS']:
            while True:
                cand = [f for f in todo if f < nmid and (fill[f][3] is None or fill[f][3] in done)]
                if not cand or acc[1] + fill[cand[0]][2] * cfg['BIAS'] > acc[0] * tot_b / tot_f:
                    break
                emit(cand[0])
        if tag is not None:
            for f in [f for f in todo if fill[f][4] == tag]:
                emit(f)
        if k >= first:
            acc[0] += it[2]
        out.append(it)
        done.add(tag)
    for f in list(todo):
        emit(f)
    return out


def _phase(R, base, z, cfg, a=None, b=None, c=None, akw={}, bkw={}, ckw={}, extra=()):
    parts = {}
    if a is not None:
        parts.update(_a_items(R, None, base, a[0], a[1], cfg, **akw))
    if c is not None:
        parts.update(_c_items(R, base, c[0], c[1], **ckw))
    fill = list(extra)
    for key in cfg['ORDER'].split(','):
        fill += parts.get(key, [])
    pre = parts.get('ln', [])
    if b is None:
        return pre + fill
    return pre + _merge(_b_items(R, base, b[0], b[1], cfg, z, **bkw), fill, cfg)


def _kernel(x_hbm, wqkv_hbm, wo_hbm, w1_hbm, b1_ref, w2_hbm, b2_ref, o_hbm,
            x_ref, o_ref, kg_ref, vt_ref, wvt_ref, wq_ref, wk_ref, wv_ref, wo_ref, w1_ref, w2_ref,
            p0_ref, p1_ref, p2_ref, z_ref,
            xn0, xn1, xs0, xs1, g0, g1, q_ref, s_ref, ot_ref, h1_ref, hn_ref,
            qa_ref, h1a_ref, hna_ref,
            sem, xsem, osem, *, cfg):
    i = pl.program_id(0)
    R = _Refs()
    R.x, R.o, R.kg, R.vt, R.wvt = x_ref, o_ref, kg_ref, vt_ref, wvt_ref
    R.wq, R.wk, R.wo, R.w1, R.w2, R.b1, R.b2 = wq_ref, wk_ref, wo_ref, w1_ref, w2_ref, b1_ref, b2_ref
    R.p = (p0_ref, p1_ref, p2_ref)
    R.xn, R.xs, R.g = (xn0, xn1), (xs0, xs1), (g0, g1)
    R.q, R.s, R.ot = q_ref, s_ref, ot_ref
    R.h1, R.hn = (h1_ref, h1a_ref), (hn_ref, hna_ref)
    only = cfg['ONLY']
    gcfg = cfg

    def rcfg(name):
        c = dict(gcfg)
        c.update(gcfg.get(name) or {})
        return c

    class _Multi:
        def __init__(self, n, src, c0, dst):
            rows, cols = dst.shape
            ns = cfg['NSPL'][n]
            r = rows // ns
            self.cs = [pltpu.make_async_copy(src.at[pl.ds(k * r, r), pl.ds(c0, cols)],
                                             dst.at[pl.ds(k * r, r), :], sem.at[n, k])
                       for k in range(ns)]

        def start(self):
            for c in self.cs:
                c.start()

        def wait(self):
            for c in self.cs:
                c.wait()

    copies = [_Multi(n, src, c0, dst) for n, (src, c0, dst) in enumerate(
        [(wqkv_hbm, D, wk_ref), (wqkv_hbm, 0, wq_ref), (wqkv_hbm, 2 * D, wv_ref),
         (wo_hbm, 0, wo_ref), (w1_hbm, 0, w1_ref), (w2_hbm, 0, w2_ref)])]

    def xcopy(b):
        return pltpu.make_async_copy(x_hbm.at[0, pl.ds(b * TQ, TQ), :],
                                     x_ref.at[pl.ds(b * TQ, TQ), :], xsem.at[b])

    def ocopy(b):
        return pltpu.make_async_copy(o_ref.at[pl.ds(b * TQ, TQ), :],
                                     o_hbm.at[0, pl.ds(b * TQ, TQ), :], osem.at[b])

    def static_base(u):
        return dict(krow=u * (TQ // 2), xrow=u * TQ, kb=u * NB)

    @pl.when(i == 0)
    def _first():
        if only not in (None, 'first'):
            return
        cfg = rcfg('first')
        plan = cfg['PLAN']

        def go(p):
            for name in plan[p].split():
                if name[0] == 'x':
                    xcopy(int(name[1:])).start()
                else:
                    copies['kqvo12'.index(name)].start()

        go(0)
        z_ref[0] = 0
        lane1 = lax.broadcasted_iota(i32, (W // 2, 128), 1)
        for g in range(NG):
            sp = (80 * g + 80) % 128
            kg_ref[g, 0:W // 2, :] = jnp.where(lane1 == sp, ONE_WORD, 0).astype(i32)
        vt_ref[0:2] = jnp.zeros((2, H * 16, 128), i32)
        xcopy(0).wait()
        go(1)
        base = static_base(0)
        a0 = _a_items(R, None, base, 0, 0, cfg, q_ref=qa_ref)
        a0['ln'][0][1]()
        copies[0].wait()
        go(2)
        for it in a0['k']:
            it[1]()
        copies[1].wait()
        go(3)
        if cfg['MERGEW']:
            copies[2].wait()
            xcopy(1).wait()
            go(4)
        for it in a0['q']:
            it[1]()
        if not cfg['MERGEW']:
            copies[2].wait()
            xcopy(1).wait()
            go(4)
        wvt_ref[...] = wv_ref[...].astype(f32).T.astype(bf16)
        z = z_ref[0]
        items = _phase(R, base, z, cfg, a=(1, 1), b=(0, 0), akw=dict(free=True),
                       bkw=dict(q_ref=qa_ref))
        k = next(n for n, it in enumerate(items) if it[0] == 'pv')
        items = items[:k] + a0['v'] + items[k:]
        k = next(n for n, it in enumerate(items) if it[0] == 'wo') - cfg['WOW']
        for n, it in enumerate(items):
            if n == k:
                copies[3].wait()
                go(5)
            it[1]()
        go(6)
        copies[4].wait()
        copies[5].wait()

    @pl.when((i > 0) & (i < NU - 1))
    def _mid():
        if only not in (None, 'mid'):
            return
        cfg = rcfg('mid')
        xcopy(i + 1).wait()
        base = dict(krow=pl.multiple_of((i - 1) * (TQ // 2), TQ // 2),
                    xrow=pl.multiple_of((i - 1) * TQ, TQ), kb=(i - 1) * NB)
        z = z_ref[0]
        for it in _phase(R, base, z, cfg, a=(2, 0), b=(1, 0), c=(0, 0)):
            it[1]()
        ocopy(i - 1).start()

    @pl.when(i == NU - 1)
    def _last():
        if only not in (None, 'last'):
            return
        cfg = rcfg('last')
        base = static_base(NU - 2)
        z = z_ref[0]
        for it in _phase(R, base, z, cfg, b=(1, 0), c=(0, 0), bkw=dict(hbuf=1), ckw=dict(free=True)):
            it[1]()
        ocopy(NU - 2).start()
        r0 = (NU - 1) * TQ
        pieces = {16: (r0, 128, 0, D), 16 + cfg['OSPL']: (r0 + 128, 128, 0, 128 * cfg['OSPL']),
                  21: (r0 + 128, 128, 128 * cfg['OSPL'], D - 128 * cfg['OSPL'])}
        tail = []
        for n, it in enumerate(_phase(R, base, z, cfg, c=(1, 1), ckw=dict(hbuf=1))):
            it[1]()
            if n in pieces:
                r, nr, c, nc = pieces[n]
                cp = pltpu.make_async_copy(o_ref.at[pl.ds(r, nr), pl.ds(c, nc)],
                                           o_hbm.at[0, pl.ds(r, nr), pl.ds(c, nc)],
                                           osem.at[NU - 1 + len(tail)])
                cp.start()
                tail.append(cp)
        for b in range(NU - 1):
            ocopy(b).wait()
        for cp in tail:
            cp.wait()


def make(**kw):
    cfg = dict(DEFAULT_CFG)
    cfg.update(kw)

    @jax.jit
    def fn(A_x, A_wqkv, A_wo, B_x, B_w1, B_b1, B_w2, B_b2):
        del B_x
        hbm = pl.BlockSpec(memory_space=pl.ANY)
        two = lambda shape, dt: [pltpu.VMEM(shape, dt)] * 2
        return pl.pallas_call(
            functools.partial(_kernel, cfg=cfg),
            grid=(NU,),
            in_specs=[
                hbm, hbm, hbm, hbm,
                pl.BlockSpec((F,), lambda i: (0,)),
                hbm,
                pl.BlockSpec((D,), lambda i: (0,)),
            ],
            out_specs=hbm,
            out_shape=jax.ShapeDtypeStruct((1, S, D), bf16),
            scratch_shapes=[
                pltpu.VMEM((S, D), bf16),
                pltpu.VMEM((S, D), bf16),
                pltpu.VMEM((NG, (S + W) // 2, 128), i32),
                pltpu.VMEM((S // 128 + 2, H * 16, 128), i32),
                pltpu.VMEM((D, D), bf16),
                pltpu.VMEM((D, D), bf16),
                pltpu.VMEM((D, D), bf16),
                pltpu.VMEM((D, D), bf16),
                pltpu.VMEM((D, D), bf16),
                pltpu.VMEM((D, F), bf16),
                pltpu.VMEM((F, D), bf16),
                pltpu.VMEM((5, 128, 128), i32),
                pltpu.VMEM((5, 128, 128), i32),
                pltpu.VMEM((5, 128, 128), i32),
                pltpu.SMEM((1,), i32),
            ] + two((TQ // 2, D), i32) + two((TQ // 2, D), i32) + two((TQ // 2, F), i32) + [
                pltpu.VMEM((NG, TQ // 2, 128), i32),
                pltpu.VMEM((TQ // 4, 256, 128), f32),
                pltpu.VMEM((NB, D, 128), f32),
                pltpu.VMEM((TQ, D), f32),
                pltpu.VMEM((TQ // 2, D), i32),
                pltpu.VMEM((NG, TQ // 2, 128), i32),
                pltpu.VMEM((TQ, D), f32),
                pltpu.VMEM((TQ // 2, D), i32),
                pltpu.SemaphoreType.DMA((6, 8)),
                pltpu.SemaphoreType.DMA((NU,)),
                pltpu.SemaphoreType.DMA((NU + 2,)),
            ],
            compiler_params=pltpu.CompilerParams(
                dimension_semantics=("arbitrary",),
                vmem_limit_bytes=100 * 2**20),
        )(A_x, A_wqkv, A_wo, B_w1, B_b1, B_w2, B_b2)
    return fn


pallas_sequential_preLN__sliding_block__dense_activation_gelu__prompt_kernel = make()
```

```python
import functools
import math

import jax
import jax.numpy as jnp
from jax import lax
import jax.experimental.pallas as pl
import jax.experimental.pallas.tpu as pltpu

S = 2048
D = 640
F = 1536
H = 32
DH = 20
W = 256
NG = 8
TQ = 256
NB = TQ // 128
NU = S // TQ
EPS = 1e-5
QSCALE = (DH ** -0.5) * math.log2(math.e)
NEG_WORD = -243207808
ONE_WORD = 0x3F803F80

f32 = jnp.float32
bf16 = jnp.bfloat16
i32 = jnp.int32

DEFAULT_CFG = dict(
    DEPTH=2,
    REL=((0, 0), (0, 96), (0, 200)),
    SS=16, SD=2,
    WOD=2,
    INS=('pv',),
    TAIL=(2, 2),
    START=1,
    VCH=4,
    ORDER='f1,f2a,k,v,f2b,q',
    BIAS=0.5,
    ONLY=None,
    PLAN=dict(start='x0 ka', x0='kb', ka='qa qb', kb='v x1', qa='w1 w2 o', v='x2', o='x3', end='x4 x5 x6 x7'),
    KS=2, QS=5, WV=2, PVS=0,
    WOW=2,
    MERGEW=0,
    OSPL=4,
    first=dict(DEPTH=2, REL=(None, (0, 96), (0, 168)), WOD=3, INS=('pv', 'qk'), TAIL=(0, 3),
               START=3, VCH=4, ORDER='k,f1,f2a,v,f2b,q', BIAS=1.0, WV=2, WOW=2),
    mid=dict(DEPTH=2, REL=(None, (1, 96), (0, 144)), WOD=3, INS=('pv', 'qk'), TAIL=(1, 4),
             START=1, VCH=8, ORDER='f1,f2a,f2b,k,v,q', BIAS=1.0),
    last=dict(DEPTH=1, REL=((0, 24), (0, 96), (0, 144)), WOD=3, INS=('pv',), TAIL=(1, 2),
              START=1, VCH=4, ORDER='f1,f2a,f2b,k,v,q', BIAS=0.0),
)


def _ln(x):
    m = jnp.mean(x, axis=-1, keepdims=True)
    xc = x - m
    v = jnp.mean(xc * xc, axis=-1, keepdims=True)
    return xc * lax.rsqrt(v + EPS)


def _gelu(x):
    c = math.sqrt(2.0 / math.pi)
    return 0.5 * x * (1.0 + jnp.tanh(c * (x + 0.044715 * (x * x * x))))


def _pack_i(a):
    R, C = a.shape
    a3 = a.reshape(R // 16, 16, C)
    w = pltpu.pack_elementwise([a3[:, 0:8, :], a3[:, 8:16, :]], packed_dtype=bf16)
    return w.reshape(R // 2, C)


def _words(a):
    return pltpu.bitcast(a.astype(bf16), i32)


def _as_bf16(w):
    return pltpu.bitcast(w, bf16)


def _group_tile(tiles, g, lane, zero_rest):
    lo = 80 * g
    t, off = lo // 128, lo % 128
    if off + 80 <= 128:
        if zero_rest:
            return jnp.where((lane >= off) & (lane < off + 80), tiles[t], 0)
        return tiles[t]
    e = off + 80 - 128
    if zero_rest:
        return jnp.where(lane < e, tiles[t + 1], jnp.where(lane >= off, tiles[t], 0))
    return jnp.where(lane < e, tiles[t + 1], tiles[t])


def _groups_ready(t):
    return [g for g in range(NG) if (80 * g + 79) // 128 == t]


def _sel(m, t, f_):
    if t is None and f_ is None:
        return None
    if t is None:
        t = 0
    if f_ is None:
        f_ = 0
    return jnp.where(m, t, f_)


class _Refs:
    pass


def _a_items(R, u, base, du, par, cfg, q_ref=None, free=False):
    st = {}
    xn_ref, xs_ref = R.xn[par], R.xs[par]
    q_ref = R.q if q_ref is None else q_ref
    row0 = base['krow'] + du * (TQ // 2)

    def ln1():
        x = R.x[pl.ds(base['xrow'] + du * TQ, TQ), :].astype(f32)
        xnf = _ln(x)
        xn_ref[...] = _words(xnf)
        xs_ref[...] = _pack_i(xnf)

    def kproj(t):
        k = jnp.dot(_as_bf16(xn_ref[...]), R.wk[:, 128 * t:128 * t + 128],
                    preferred_element_type=f32)
        st[('k', t)] = _words(k)
        lane = lax.broadcasted_iota(i32, (TQ // 2, 128), 1)
        tiles = {tt: st[('k', tt)] for tt in range(t + 1)}
        for g in _groups_ready(t):
            R.kg[g, pl.ds(row0 + W // 2, TQ // 2), :] = _group_tile(tiles, g, lane, True)

    def qproj(t):
        q = jnp.dot(_as_bf16(xn_ref[...]), R.wq[:, 128 * t:128 * t + 128],
                    preferred_element_type=f32) * QSCALE
        st[('q', t)] = _words(q)
        lane = lax.broadcasted_iota(i32, (TQ // 2, 128), 1)
        tiles = {tt: st[('q', tt)] for tt in range(t + 1)}
        for g in _groups_ready(t):
            q_ref[g] = _group_tile(tiles, g, lane, False)

    def vproj(c):
        gpc = NG // cfg['VCH']
        m0 = 80 * gpc * c
        vt = lax.dot_general(R.wvt[m0:m0 + 80 * gpc, :], _as_bf16(xs_ref[...]),
                             (((1,), (1,)), ((), ())), preferred_element_type=f32)
        vtw = _words(vt)
        sub8 = lax.broadcasted_iota(i32, (8, TQ), 0)
        pieces = []
        for gg in range(gpc):
            for hh in range(4):
                w0 = 40 * gg + 8 * hh
                a = vtw[w0:w0 + 8]
                b = vtw[w0 + 8:w0 + 16]
                if hh < 2:
                    b = jnp.where(sub8 >= 4, ONE_WORD, b)
                else:
                    a = jnp.where(sub8 < 4, ONE_WORD, a)
                pieces += [a, b]
        vtp = jnp.concatenate(pieces, axis=0)
        for nb in range(NB):
            R.vt[base['kb'] + du * NB + nb + 2, 64 * gpc * c:64 * gpc * (c + 1), :] = (
                vtp[:, 128 * nb:128 * nb + 128])

    return dict(
        ln=[('ln1', ln1, 0)],
        k=[('k', functools.partial(kproj, t), 320) for t in range(5)],
        q=[('q', functools.partial(qproj, t), 320, None if free else ('qk', NG + max(_groups_ready(t))), None)
           for t in range(5)],
        v=[('v', functools.partial(vproj, c), 1600 // cfg['VCH']) for c in range(cfg['VCH'])],
    )


def _b_items(R, base, du, par, cfg, z, q_ref=None, hbuf=0):
    st = {}
    s_ref, ot_ref = R.s, R.ot
    q_ref = R.q if q_ref is None else q_ref
    h1_ref, hn_ref = R.h1[hbuf], R.hn[hbuf]
    row0 = base['krow'] + du * (TQ // 2)
    DEPTH, SS, SD = cfg['DEPTH'], cfg['SS'], cfg['SD']

    lane16 = lax.broadcasted_iota(i32, (16, 128), 1)
    r16 = lax.broadcasted_iota(i32, (16, 128), 0)
    cw = lane16 & 31
    tri0 = r16 > cw
    tri1 = r16 + 16 > cw
    rw = (r16 & 7) + 2 * (r16 & 8)
    m_old = (jnp.where(rw > cw, 0xFFFF, 0) | jnp.where(rw + 8 > cw, -65536, 0)).astype(i32)
    m_new = ~m_old
    s_odd = (lane16 & 32) != 0
    s_hi = (lane16 & 64) != 0
    sub8b = lax.broadcasted_iota(i32, (8, 128), 0) < 4

    def qk_stage(n):
        nb, g = n // NG, n % NG
        off = (80 * g) % 128
        rel = (lane16 - off) & 127
        cneg = jnp.where(rel == 80, NEG_WORD, 0).astype(i32)
        hmask = [(rel >= 20 * hh) & (rel < 20 * hh + 20) for hh in range(4)]
        for j in range(4):
            jj = 4 * nb + j
            qs = q_ref[g, 16 * jj:16 * jj + 16, :]
            bmat = _as_bf16(jnp.concatenate(
                [jnp.where(hmask[s ^ j], qs, cneg) for s in range(4)], axis=0))
            kw = R.kg[g, pl.ds(row0 + 16 * jj, 144), :]
            kwin = _as_bf16(jnp.concatenate(
                [kw[16:128], kw[0:8], kw[128:136], kw[8:16], kw[136:144]], axis=0))
            s_t = lax.dot_general(kwin, bmat, (((1,), (1,)), ((), ())),
                                  preferred_element_type=f32)
            slot = n * 4 + j
            e0 = jnp.where(tri0, s_t[224:240], s_t[240:256])
            e1 = jnp.where(tri1, s_t[256:272], s_t[272:288])
            sm = jnp.concatenate([s_t[0:224], e0, e1], axis=0)
            m = None
            for r in range(0, 256, 8):
                v = sm[r:r + 8]
                if m is None:
                    m = v
                    s_ref[slot, r:r + 8, :] = v
                else:
                    m = jnp.maximum(m, v)
                    s_ref[slot, r:r + 8, :] = jnp.minimum(v, m)
            st[('mx', n, j)] = jnp.max(m, axis=0, keepdims=True)
            st[('st', n, j)] = s_t

    def sm_stage(n):
        for j in range(4):
            slot = n * 4 + j
            mx = jnp.broadcast_to(st.pop(('mx', n, j)), (8, 128))
            hist = []
            for r in range(0, 256, SS):
                if len(hist) >= SD:
                    mx = jnp.maximum(mx, hist[-SD] - 3e38)
                p = jnp.exp2(s_ref[slot, r:r + SS, :] - jnp.concatenate([mx] * (SS // 8), axis=0))
                hist.append(p[SS - 8:SS])
                R.p[n % 3][j, r // 2:(r + SS) // 2, :] = _pack_i(p)

    def pv_stage(n, ts=(0, 1, 2)):
        nb, g = n // NG, n % NG
        p_ref = R.p[n % 3]
        kb = base['kb'] + du * NB + nb
        acc = st.setdefault(('acc', n), [None] * 4)
        for t in ts:
            spec = cfg['REL'][t]
            if spec is not None and ('st', n + DEPTH, spec[0]) in st:
                s_t = st[('st', n + DEPTH, spec[0])]
                p_ref[4, 8 * t:8 * t + 8, :] = pltpu.bitcast(s_t[spec[1]:spec[1] + 8], i32)

            def blk(j, b):
                if b < 0 or b > 8:
                    return None
                if b == 0:
                    return p_ref[z + j, 112:128, :] & m_old
                if b == 8:
                    return p_ref[z + j, 112:128, :] & m_new
                return p_ref[z + j, 16 * (b - 1):16 * b, :]

            wrows = [[], [], [], []]
            for a in range(4 * t, 4 * t + 4):
                X = [blk(j, a - j) for j in range(4)]
                Y = [_sel(s_odd, X[1], X[0]), _sel(s_odd, X[0], X[1]),
                     _sel(s_odd, X[3], X[2]), _sel(s_odd, X[2], X[3])]
                Z = [_sel(s_hi, Y[2], Y[0]), _sel(s_hi, Y[3], Y[1]),
                     _sel(s_hi, Y[0], Y[2]), _sel(s_hi, Y[1], Y[3])]
                for hh in range(4):
                    wrows[hh].append(Z[hh])
            for hh in range(4):
                h = 4 * g + hh
                wm = _as_bf16(jnp.concatenate(wrows[hh], axis=0))
                vl = _as_bf16(R.vt[kb + t, 16 * h:16 * h + 16, :])
                ot = jnp.dot(vl, wm, preferred_element_type=f32)
                acc[hh] = ot if acc[hh] is None else acc[hh] + ot
        if 2 not in ts:
            return
        on = []
        for hh in range(4):
            ot = acc[hh]
            den = ot[24:32] if hh < 2 else ot[0:8]
            r = 1.0 / den
            on.append([ot[8 * t:8 * t + 8] * r for t in range(4)])
        ot_ref[nb, 80 * g:80 * g + 80, :] = jnp.concatenate(
            [on[0][0], on[0][1], jnp.where(sub8b, on[0][2], on[1][0]),
             on[1][1], on[1][2], on[2][1], on[2][2],
             jnp.where(sub8b, on[2][3], on[3][1]), on[3][2], on[3][3]], axis=0)

    def wo_stage(nb):
        t = ot_ref[nb].T
        lane640 = lax.broadcasted_iota(i32, (32, D), 1)
        hid = lane640 // DH
        b0 = (hid & 1) != 0
        b1 = (hid & 2) != 0
        X = [t[32 * j:32 * j + 32] for j in range(4)]
        Y = [jnp.where(b0, X[j ^ 1], X[j]) for j in range(4)]
        Z = [jnp.where(b1, Y[j ^ 2], Y[j]) for j in range(4)]
        o = jnp.concatenate(Z, axis=0).astype(bf16)
        x = R.x[pl.ds(base['xrow'] + du * TQ + 128 * nb, 128), :].astype(f32)
        h1 = x + jnp.dot(o, R.wo[...], preferred_element_type=f32)
        h1_ref[128 * nb:128 * nb + 128, :] = h1
        hn_ref[64 * nb:64 * nb + 64, :] = _words(_ln(h1))

    items = []
    NA = NB * NG
    pend = []
    for n in range(NA + DEPTH):
        if n < NA:
            items.append(('qk', functools.partial(qk_stage, n), 288, n))
            items.append(('sm', functools.partial(sm_stage, n), 0))
        m = n - DEPTH
        if m >= 0:
            if cfg['PVS'] == 0:
                items.append(('pv', functools.partial(pv_stage, m), 96))
            elif cfg['PVS'] == 1:
                items.append(('pv', functools.partial(pv_stage, m, (0, 1)), 64))
                items.append(('pw', functools.partial(pv_stage, m, (2,)), 32))
            elif cfg['PVS'] == 2:
                items.append(('pv', functools.partial(pv_stage, m, (0,)), 32))
                items.append(('pw', functools.partial(pv_stage, m, (1,)), 32))
                items.append(('pw', functools.partial(pv_stage, m, (2,)), 32))
            if pend and n >= pend[0][0]:
                items.append(pend.pop(0)[1])
            if m % NG == NG - 1:
                pend.append((n + cfg['WOD'], ('wo', functools.partial(wo_stage, m // NG), 800, m // NG)))
    items += [w[1] for w in pend]
    return items


def _c_items(R, base, du, par, hbuf=0, free=False):
    h1_ref, hn_ref, g_ref = R.h1[hbuf], R.hn[hbuf], R.g[par]
    w0, w1 = (None, None) if free else (('wo', 0), ('wo', 1))

    def f1(c):
        u = jnp.dot(_as_bf16(hn_ref[...]), R.w1[:, 128 * c:128 * c + 128],
                    preferred_element_type=f32)
        u = u + R.b1[128 * c:128 * c + 128].astype(f32).reshape(1, 128)
        g_ref[:, 128 * c:128 * c + 128] = _words(_gelu(u))

    def f2(m, n):
        g = _as_bf16(g_ref[64 * m:64 * m + 64, :])
        y = jnp.dot(g, R.w2[:, 128 * n:128 * n + 128], preferred_element_type=f32)
        y = y + R.b2[128 * n:128 * n + 128].astype(f32).reshape(1, 128)
        R.o[pl.ds(base['xrow'] + du * TQ + 128 * m, 128), 128 * n:128 * n + 128] = (
            h1_ref[128 * m:128 * m + 128, 128 * n:128 * n + 128] + y).astype(bf16)

    return dict(
        f1=[('f1', functools.partial(f1, c), 320, None, w0) for c in range(F // 128)],
        f2a=[('f2', functools.partial(f2, 0, n), 384, None, w0) for n in range(D // 128)],
        f2b=[('f2', functools.partial(f2, 1, n), 384, None, w1) for n in range(D // 128)],
    )


def _merge(main, fill, cfg):
    fill = [it if len(it) == 5 else it + (None, None) for it in fill]
    t1, t2 = cfg['TAIL']
    t2 = min(t2, len(fill))
    t1 = min(t1, len(fill) - t2)
    nmid = len(fill) - t1 - t2
    first = cfg['START']
    tot_f = sum(it[2] for it in main[first:-1])
    tot_b = sum(it[2] for it in fill[:nmid])
    out, done = [], set()
    todo = list(range(len(fill)))
    acc = [0, 0]

    def emit(k):
        todo.remove(k)
        out.append(fill[k])
        acc[1] += fill[k][2]

    for k, it in enumerate(main):
        tag = (it[0], it[3]) if len(it) > 3 else None
        if k == len(main) - 1:
            for f in [f for f in todo if f < nmid + t1]:
                emit(f)
        elif k >= first and it[0] in cfg['INS']:
            while True:
                cand = [f for f in todo if f < nmid and (fill[f][3] is None or fill[f][3] in done)]
                if not cand or acc[1] + fill[cand[0]][2] * cfg['BIAS'] > acc[0] * tot_b / tot_f:
                    break
                emit(cand[0])
        if tag is not None:
            for f in [f for f in todo if fill[f][4] == tag]:
                emit(f)
        if k >= first:
            acc[0] += it[2]
        out.append(it)
        done.add(tag)
    for f in list(todo):
        emit(f)
    return out


def _phase(R, base, z, cfg, a=None, b=None, c=None, akw={}, bkw={}, ckw={}, extra=()):
    parts = {}
    if a is not None:
        parts.update(_a_items(R, None, base, a[0], a[1], cfg, **akw))
    if c is not None:
        parts.update(_c_items(R, base, c[0], c[1], **ckw))
    fill = list(extra)
    for key in cfg['ORDER'].split(','):
        fill += parts.get(key, [])
    pre = parts.get('ln', [])
    if b is None:
        return pre + fill
    return pre + _merge(_b_items(R, base, b[0], b[1], cfg, z, **bkw), fill, cfg)


def _kernel(x_hbm, wqkv_hbm, wo_hbm, w1_hbm, b1_ref, w2_hbm, b2_ref, o_hbm,
            x_ref, o_ref, kg_ref, vt_ref, wvt_ref, wq_ref, wk_ref, wv_ref, wo_ref, w1_ref, w2_ref,
            p0_ref, p1_ref, p2_ref, z_ref,
            xn0, xn1, xs0, xs1, g0, g1, q_ref, s_ref, ot_ref, h1_ref, hn_ref,
            qa_ref, h1a_ref, hna_ref,
            sem, xsem, osem, *, cfg):
    i = pl.program_id(0)
    R = _Refs()
    R.x, R.o, R.kg, R.vt, R.wvt = x_ref, o_ref, kg_ref, vt_ref, wvt_ref
    R.wq, R.wk, R.wo, R.w1, R.w2, R.b1, R.b2 = wq_ref, wk_ref, wo_ref, w1_ref, w2_ref, b1_ref, b2_ref
    R.p = (p0_ref, p1_ref, p2_ref)
    R.xn, R.xs, R.g = (xn0, xn1), (xs0, xs1), (g0, g1)
    R.q, R.s, R.ot = q_ref, s_ref, ot_ref
    R.h1, R.hn = (h1_ref, h1a_ref), (hn_ref, hna_ref)
    only = cfg['ONLY']
    gcfg = cfg

    def rcfg(name):
        c = dict(gcfg)
        c.update(gcfg.get(name) or {})
        return c

    KS, QS = cfg['KS'], cfg['QS']
    specs = dict(
        ka=(wqkv_hbm, D, wk_ref, 0, 128 * KS), kb=(wqkv_hbm, D, wk_ref, 128 * KS, D - 128 * KS),
        qa=(wqkv_hbm, 0, wq_ref, 0, 128 * QS), qb=(wqkv_hbm, 0, wq_ref, 128 * QS, D - 128 * QS),
        v=(wqkv_hbm, 2 * D, wv_ref, 0, D), o=(wo_hbm, 0, wo_ref, 0, D),
        w1=(w1_hbm, 0, w1_ref, 0, F), w2=(w2_hbm, 0, w2_ref, 0, D))
    copies = {}
    for n, (name, (src, c0, dst, d0, nc)) in enumerate(specs.items()):
        if nc > 0:
            copies[name] = pltpu.make_async_copy(
                src.at[:, pl.ds(c0 + d0, nc)], dst.at[:, pl.ds(d0, nc)], sem.at[n])

    def xcopy(b):
        return pltpu.make_async_copy(x_hbm.at[0, pl.ds(b * TQ, TQ), :],
                                     x_ref.at[pl.ds(b * TQ, TQ), :], xsem.at[b])

    def ocopy(b):
        return pltpu.make_async_copy(o_ref.at[pl.ds(b * TQ, TQ), :],
                                     o_hbm.at[0, pl.ds(b * TQ, TQ), :], osem.at[b])

    def static_base(u):
        return dict(krow=u * (TQ // 2), xrow=u * TQ, kb=u * NB)

    @pl.when(i == 0)
    def _first():
        if only not in (None, 'first'):
            return
        cfg = rcfg('first')
        plan = cfg['PLAN']

        def go(p):
            for name in plan.get(p, '').split():
                if name[0] == 'x':
                    xcopy(int(name[1:])).start()
                elif name in copies:
                    copies[name].start()

        def wait(name):
            if name in copies:
                copies[name].wait()
            go(name)

        go('start')
        z_ref[0] = 0
        lane1 = lax.broadcasted_iota(i32, (W // 2, 128), 1)
        for g in range(NG):
            sp = (80 * g + 80) % 128
            kg_ref[g, 0:W // 2, :] = jnp.where(lane1 == sp, ONE_WORD, 0).astype(i32)
        vt_ref[0:2] = jnp.zeros((2, H * 16, 128), i32)
        xcopy(0).wait()
        go('x0')
        base = static_base(0)
        a0 = _a_items(R, None, base, 0, 0, cfg, q_ref=qa_ref)
        a0['ln'][0][1]()
        wait('ka')
        for it in a0['k'][:KS]:
            it[1]()
        wait('kb')
        for it in a0['k'][KS:]:
            it[1]()
        wait('qa')
        for it in a0['q'][:QS]:
            it[1]()
        wait('qb')
        for it in a0['q'][QS:]:
            it[1]()
        z = z_ref[0]
        items = _phase(R, base, z, cfg, a=(1, 1), b=(0, 0), akw=dict(free=True),
                       bkw=dict(q_ref=qa_ref))

        def vwait():
            xcopy(1).wait()
            wait('v')
            wvt_ref[...] = wv_ref[...].astype(f32).T.astype(bf16)

        ln1, items = items[0], items[1:]
        lead = [it for it in items if it[0] in ('qk', 'sm')][:2 * cfg['WV']]
        items = [it for it in items if not any(it is l for l in lead)]
        k = next(n for n, it in enumerate(items) if it[0] == 'pv')
        items = lead + [('w', vwait), ln1] + items[:k] + a0['v'] + items[k:]
        k = next(n for n, it in enumerate(items) if it[0] == 'wo') - cfg['WOW']
        for n, it in enumerate(items):
            if n == k:
                wait('o')
            it[1]()
        go('end')
        wait('w1')
        wait('w2')

    @pl.when((i > 0) & (i < NU - 1))
    def _mid():
        if only not in (None, 'mid'):
            return
        cfg = rcfg('mid')
        xcopy(i + 1).wait()
        base = dict(krow=pl.multiple_of((i - 1) * (TQ // 2), TQ // 2),
                    xrow=pl.multiple_of((i - 1) * TQ, TQ), kb=(i - 1) * NB)
        z = z_ref[0]
        for it in _phase(R, base, z, cfg, a=(2, 0), b=(1, 0), c=(0, 0)):
            it[1]()
        ocopy(i - 1).start()

    @pl.when(i == NU - 1)
    def _last():
        if only not in (None, 'last'):
            return
        cfg = rcfg('last')
        base = static_base(NU - 2)
        z = z_ref[0]
        for it in _phase(R, base, z, cfg, b=(1, 0), c=(0, 0), bkw=dict(hbuf=1), ckw=dict(free=True)):
            it[1]()
        ocopy(NU - 2).start()
        r0 = (NU - 1) * TQ
        pieces = {16: (r0, 128, 0, D), 16 + cfg['OSPL']: (r0 + 128, 128, 0, 128 * cfg['OSPL']),
                  21: (r0 + 128, 128, 128 * cfg['OSPL'], D - 128 * cfg['OSPL'])}
        tail = []
        for n, it in enumerate(_phase(R, base, z, cfg, c=(1, 1), ckw=dict(hbuf=1))):
            it[1]()
            if n in pieces:
                r, nr, c, nc = pieces[n]
                cp = pltpu.make_async_copy(o_ref.at[pl.ds(r, nr), pl.ds(c, nc)],
                                           o_hbm.at[0, pl.ds(r, nr), pl.ds(c, nc)],
                                           osem.at[NU - 1 + len(tail)])
                cp.start()
                tail.append(cp)
        for b in range(NU - 1):
            ocopy(b).wait()
        for cp in tail:
            cp.wait()


def make(**kw):
    cfg = dict(DEFAULT_CFG)
    cfg.update(kw)

    @jax.jit
    def fn(A_x, A_wqkv, A_wo, B_x, B_w1, B_b1, B_w2, B_b2):
        del B_x
        hbm = pl.BlockSpec(memory_space=pl.ANY)
        two = lambda shape, dt: [pltpu.VMEM(shape, dt)] * 2
        return pl.pallas_call(
            functools.partial(_kernel, cfg=cfg),
            grid=(NU,),
            in_specs=[
                hbm, hbm, hbm, hbm,
                pl.BlockSpec((F,), lambda i: (0,)),
                hbm,
                pl.BlockSpec((D,), lambda i: (0,)),
            ],
            out_specs=hbm,
            out_shape=jax.ShapeDtypeStruct((1, S, D), bf16),
            scratch_shapes=[
                pltpu.VMEM((S, D), bf16),
                pltpu.VMEM((S, D), bf16),
                pltpu.VMEM((NG, (S + W) // 2, 128), i32),
                pltpu.VMEM((S // 128 + 2, H * 16, 128), i32),
                pltpu.VMEM((D, D), bf16),
                pltpu.VMEM((D, D), bf16),
                pltpu.VMEM((D, D), bf16),
                pltpu.VMEM((D, D), bf16),
                pltpu.VMEM((D, D), bf16),
                pltpu.VMEM((D, F), bf16),
                pltpu.VMEM((F, D), bf16),
                pltpu.VMEM((5, 128, 128), i32),
                pltpu.VMEM((5, 128, 128), i32),
                pltpu.VMEM((5, 128, 128), i32),
                pltpu.SMEM((1,), i32),
            ] + two((TQ // 2, D), i32) + two((TQ // 2, D), i32) + two((TQ // 2, F), i32) + [
                pltpu.VMEM((NG, TQ // 2, 128), i32),
                pltpu.VMEM((TQ // 4, 256, 128), f32),
                pltpu.VMEM((NB, D, 128), f32),
                pltpu.VMEM((TQ, D), f32),
                pltpu.VMEM((TQ // 2, D), i32),
                pltpu.VMEM((NG, TQ // 2, 128), i32),
                pltpu.VMEM((TQ, D), f32),
                pltpu.VMEM((TQ // 2, D), i32),
                pltpu.SemaphoreType.DMA((8,)),
                pltpu.SemaphoreType.DMA((NU,)),
                pltpu.SemaphoreType.DMA((NU + 2,)),
            ],
            compiler_params=pltpu.CompilerParams(
                dimension_semantics=("arbitrary",),
                vmem_limit_bytes=100 * 2**20),
        )(A_x, A_wqkv, A_wo, B_w1, B_b1, B_w2, B_b2)
    return fn


pallas_sequential_preLN__sliding_block__dense_activation_gelu__prompt_kernel = make()
```

```python
import functools
import math

import jax
import jax.numpy as jnp
from jax import lax
import jax.experimental.pallas as pl
import jax.experimental.pallas.tpu as pltpu

S = 2048
D = 640
F = 1536
H = 32
DH = 20
W = 256
NG = 8
TQ = 256
NB = TQ // 128
NU = S // TQ
EPS = 1e-5
QSCALE = (DH ** -0.5) * math.log2(math.e)
NEG_WORD = -243207808
ONE_WORD = 0x3F803F80

f32 = jnp.float32
bf16 = jnp.bfloat16
i32 = jnp.int32

DEFAULT_CFG = dict(
    DEPTH=2,
    REL=((0, 0), (0, 96), (0, 200)),
    SS=16, SD=2,
    WOD=2,
    INS=('pv',),
    TAIL=(2, 2),
    START=1,
    VCH=4,
    ORDER='f1,f2a,k,v,f2b,q',
    BIAS=0.5,
    ONLY=None,
    PLAN=dict(start='x0 ka kb qa qb v x1 o w1 w2 x2 b1 b2 x3 x4 x5 x6 x7'),
    OEARLY=0,
    KS=2, QS=5, WV=2, PVS=0,
    WOW=2,
    MERGEW=0,
    OSPL=4,
    first=dict(DEPTH=2, REL=((0, 0), (0, 96), (0, 168)), WOD=3, INS=('pv', 'qk'), TAIL=(0, 3),
               START=3, VCH=4, ORDER='k,f1,f2a,v,f2b,q', BIAS=1.0, WV=2, WOW=2),
    mid=dict(DEPTH=2, REL=(None, (1, 96), (2, 200)), WOD=3, INS=('pv', 'qk'), TAIL=(1, 4),
             START=1, VCH=8, ORDER='f1,f2a,f2b,k,v,q', BIAS=1.0),
    last=dict(DEPTH=1, REL=((0, 24), (0, 96), (0, 240)), WOD=3, INS=('pv',), TAIL=(1, 2),
              START=1, VCH=4, ORDER='f1,f2a,f2b,k,v,q', BIAS=0.0),
)


def _ln(x):
    m = jnp.mean(x, axis=-1, keepdims=True)
    xc = x - m
    v = jnp.mean(xc * xc, axis=-1, keepdims=True)
    return xc * lax.rsqrt(v + EPS)


def _gelu(x):
    c = math.sqrt(2.0 / math.pi)
    return 0.5 * x * (1.0 + jnp.tanh(c * (x + 0.044715 * (x * x * x))))


def _pack_i(a):
    R, C = a.shape
    a3 = a.reshape(R // 16, 16, C)
    w = pltpu.pack_elementwise([a3[:, 0:8, :], a3[:, 8:16, :]], packed_dtype=bf16)
    return w.reshape(R // 2, C)


def _words(a):
    return pltpu.bitcast(a.astype(bf16), i32)


def _as_bf16(w):
    return pltpu.bitcast(w, bf16)


def _group_tile(tiles, g, lane, zero_rest):
    lo = 80 * g
    t, off = lo // 128, lo % 128
    if off + 80 <= 128:
        if zero_rest:
            return jnp.where((lane >= off) & (lane < off + 80), tiles[t], 0)
        return tiles[t]
    e = off + 80 - 128
    if zero_rest:
        return jnp.where(lane < e, tiles[t + 1], jnp.where(lane >= off, tiles[t], 0))
    return jnp.where(lane < e, tiles[t + 1], tiles[t])


def _groups_ready(t):
    return [g for g in range(NG) if (80 * g + 79) // 128 == t]


def _sel(m, t, f_):
    if t is None and f_ is None:
        return None
    if t is None:
        t = 0
    if f_ is None:
        f_ = 0
    return jnp.where(m, t, f_)


class _Refs:
    pass


def _a_items(R, u, base, du, par, cfg, q_ref=None, free=False):
    st = {}
    xn_ref, xs_ref = R.xn[par], R.xs[par]
    q_ref = R.q if q_ref is None else q_ref
    row0 = base['krow'] + du * (TQ // 2)

    def ln1():
        x = _as_bf16(R.x[pl.ds(base['krow'] + du * (TQ // 2), TQ // 2), :]).astype(f32)
        xnf = _ln(x)
        xn_ref[...] = _words(xnf)
        xs_ref[...] = _pack_i(xnf)

    def kproj(t):
        k = jnp.dot(_as_bf16(xn_ref[...]), _as_bf16(R.wk[:, 128 * t:128 * t + 128]),
                    preferred_element_type=f32)
        st[('k', t)] = _words(k)
        lane = lax.broadcasted_iota(i32, (TQ // 2, 128), 1)
        tiles = {tt: st[('k', tt)] for tt in range(t + 1)}
        for g in _groups_ready(t):
            R.kg[g, pl.ds(row0 + W // 2, TQ // 2), :] = _group_tile(tiles, g, lane, True)

    def qproj(t):
        q = jnp.dot(_as_bf16(xn_ref[...]), _as_bf16(R.wq[:, 128 * t:128 * t + 128]),
                    preferred_element_type=f32) * QSCALE
        st[('q', t)] = _words(q)
        lane = lax.broadcasted_iota(i32, (TQ // 2, 128), 1)
        tiles = {tt: st[('q', tt)] for tt in range(t + 1)}
        for g in _groups_ready(t):
            q_ref[g] = _group_tile(tiles, g, lane, False)

    def vproj(c):
        gpc = NG // cfg['VCH']
        m0 = 80 * gpc * c
        vt = lax.dot_general(_as_bf16(R.wvt[m0 // 2:m0 // 2 + 40 * gpc, :]), _as_bf16(xs_ref[...]),
                             (((1,), (1,)), ((), ())), preferred_element_type=f32)
        vtw = _words(vt)
        sub8 = lax.broadcasted_iota(i32, (8, TQ), 0)
        pieces = []
        for gg in range(gpc):
            for hh in range(4):
                w0 = 40 * gg + 8 * hh
                a = vtw[w0:w0 + 8]
                b = vtw[w0 + 8:w0 + 16]
                if hh < 2:
                    b = jnp.where(sub8 >= 4, ONE_WORD, b)
                else:
                    a = jnp.where(sub8 < 4, ONE_WORD, a)
                pieces += [a, b]
        vtp = jnp.concatenate(pieces, axis=0)
        for nb in range(NB):
            R.vt[base['kb'] + du * NB + nb + 2, 64 * gpc * c:64 * gpc * (c + 1), :] = (
                vtp[:, 128 * nb:128 * nb + 128])

    return dict(
        ln=[('ln1', ln1, 0)],
        k=[('k', functools.partial(kproj, t), 320) for t in range(5)],
        q=[('q', functools.partial(qproj, t), 320, None if free else ('qk', NG + max(_groups_ready(t))), None)
           for t in range(5)],
        v=[('v', functools.partial(vproj, c), 1600 // cfg['VCH']) for c in range(cfg['VCH'])],
    )


def _b_items(R, base, du, par, cfg, z, q_ref=None, hbuf=0):
    st = {}
    s_ref, ot_ref = R.s, R.ot
    q_ref = R.q if q_ref is None else q_ref
    h1_ref, hn_ref = R.h1[hbuf], R.hn[hbuf]
    row0 = base['krow'] + du * (TQ // 2)
    DEPTH, SS, SD = cfg['DEPTH'], cfg['SS'], cfg['SD']

    lane16 = lax.broadcasted_iota(i32, (16, 128), 1)
    r16 = lax.broadcasted_iota(i32, (16, 128), 0)
    cw = lane16 & 31
    tri0 = r16 > cw
    tri1 = r16 + 16 > cw
    rw = (r16 & 7) + 2 * (r16 & 8)
    m_old = (jnp.where(rw > cw, 0xFFFF, 0) | jnp.where(rw + 8 > cw, -65536, 0)).astype(i32)
    m_new = ~m_old
    s_odd = (lane16 & 32) != 0
    s_hi = (lane16 & 64) != 0
    sub8b = lax.broadcasted_iota(i32, (8, 128), 0) < 4

    def qk_stage(n):
        nb, g = n // NG, n % NG
        off = (80 * g) % 128
        rel = (lane16 - off) & 127
        cneg = jnp.where(rel == 80, NEG_WORD, 0).astype(i32)
        hmask = [(rel >= 20 * hh) & (rel < 20 * hh + 20) for hh in range(4)]
        for j in range(4):
            jj = 4 * nb + j
            qs = q_ref[g, 16 * jj:16 * jj + 16, :]
            bmat = _as_bf16(jnp.concatenate(
                [jnp.where(hmask[s ^ j], qs, cneg) for s in range(4)], axis=0))
            kw = R.kg[g, pl.ds(row0 + 16 * jj, 144), :]
            kwin = _as_bf16(jnp.concatenate(
                [kw[16:128], kw[0:8], kw[128:136], kw[8:16], kw[136:144]], axis=0))
            s_t = lax.dot_general(kwin, bmat, (((1,), (1,)), ((), ())),
                                  preferred_element_type=f32)
            slot = n * 4 + j
            e0 = jnp.where(tri0, s_t[224:240], s_t[240:256])
            e1 = jnp.where(tri1, s_t[256:272], s_t[272:288])
            sm = jnp.concatenate([s_t[0:224], e0, e1], axis=0)
            m = None
            for r in range(0, 256, 8):
                v = sm[r:r + 8]
                if m is None:
                    m = v
                    s_ref[slot, r:r + 8, :] = v
                else:
                    m = jnp.maximum(m, v)
                    s_ref[slot, r:r + 8, :] = jnp.minimum(v, m)
            st[('mx', n, j)] = jnp.max(m, axis=0, keepdims=True)
            st[('st', n, j)] = s_t

    def sm_stage(n):
        for j in range(4):
            slot = n * 4 + j
            mx = jnp.broadcast_to(st.pop(('mx', n, j)), (8, 128))
            hist = []
            for r in range(0, 256, SS):
                if len(hist) >= SD:
                    mx = jnp.maximum(mx, hist[-SD] - 3e38)
                p = jnp.exp2(s_ref[slot, r:r + SS, :] - jnp.concatenate([mx] * (SS // 8), axis=0))
                hist.append(p[SS - 8:SS])
                R.p[n % 3][j, r // 2:(r + SS) // 2, :] = _pack_i(p)

    def pv_stage(n, ts=(0, 1, 2)):
        nb, g = n // NG, n % NG
        p_ref = R.p[n % 3]
        kb = base['kb'] + du * NB + nb
        acc = st.setdefault(('acc', n), [None] * 4)
        for t in ts:
            spec = cfg['REL'][t]
            if spec is not None and ('st', n + DEPTH, spec[0]) in st:
                s_t = st[('st', n + DEPTH, spec[0])]
                p_ref[4, 8 * t:8 * t + 8, :] = pltpu.bitcast(s_t[spec[1]:spec[1] + 8], i32)

            def blk(j, b):
                if b < 0 or b > 8:
                    return None
                if b == 0:
                    return p_ref[z + j, 112:128, :] & m_old
                if b == 8:
                    return p_ref[z + j, 112:128, :] & m_new
                return p_ref[z + j, 16 * (b - 1):16 * b, :]

            wrows = [[], [], [], []]
            for a in range(4 * t, 4 * t + 4):
                X = [blk(j, a - j) for j in range(4)]
                Y = [_sel(s_odd, X[1], X[0]), _sel(s_odd, X[0], X[1]),
                     _sel(s_odd, X[3], X[2]), _sel(s_odd, X[2], X[3])]
                Z = [_sel(s_hi, Y[2], Y[0]), _sel(s_hi, Y[3], Y[1]),
                     _sel(s_hi, Y[0], Y[2]), _sel(s_hi, Y[1], Y[3])]
                for hh in range(4):
                    wrows[hh].append(Z[hh])
            for hh in range(4):
                h = 4 * g + hh
                wm = _as_bf16(jnp.concatenate(wrows[hh], axis=0))
                vl = _as_bf16(R.vt[kb + t, 16 * h:16 * h + 16, :])
                ot = jnp.dot(vl, wm, preferred_element_type=f32)
                acc[hh] = ot if acc[hh] is None else acc[hh] + ot
        if 2 not in ts:
            return
        on = []
        for hh in range(4):
            ot = acc[hh]
            den = ot[24:32] if hh < 2 else ot[0:8]
            r = 1.0 / den
            on.append([ot[8 * t:8 * t + 8] * r for t in range(4)])
        ot_ref[nb, 80 * g:80 * g + 80, :] = jnp.concatenate(
            [on[0][0], on[0][1], jnp.where(sub8b, on[0][2], on[1][0]),
             on[1][1], on[1][2], on[2][1], on[2][2],
             jnp.where(sub8b, on[2][3], on[3][1]), on[3][2], on[3][3]], axis=0)

    def wo_stage(nb):
        t = ot_ref[nb].T
        lane640 = lax.broadcasted_iota(i32, (32, D), 1)
        hid = lane640 // DH
        b0 = (hid & 1) != 0
        b1 = (hid & 2) != 0
        X = [t[32 * j:32 * j + 32] for j in range(4)]
        Y = [jnp.where(b0, X[j ^ 1], X[j]) for j in range(4)]
        Z = [jnp.where(b1, Y[j ^ 2], Y[j]) for j in range(4)]
        o = jnp.concatenate(Z, axis=0).astype(bf16)
        x = _as_bf16(R.x[pl.ds(base['krow'] + du * (TQ // 2) + 64 * nb, 64), :]).astype(f32)
        h1 = x + jnp.dot(o, _as_bf16(R.wo[...]), preferred_element_type=f32)
        h1_ref[128 * nb:128 * nb + 128, :] = h1
        hn_ref[64 * nb:64 * nb + 64, :] = _words(_ln(h1))

    items = []
    NA = NB * NG
    pend = []
    for n in range(NA + DEPTH):
        if n < NA:
            items.append(('qk', functools.partial(qk_stage, n), 288, n))
            items.append(('sm', functools.partial(sm_stage, n), 0))
        m = n - DEPTH
        if m >= 0:
            if cfg['PVS'] == 0:
                items.append(('pv', functools.partial(pv_stage, m), 96))
            elif cfg['PVS'] == 1:
                items.append(('pv', functools.partial(pv_stage, m, (0, 1)), 64))
                items.append(('pw', functools.partial(pv_stage, m, (2,)), 32))
            elif cfg['PVS'] == 2:
                items.append(('pv', functools.partial(pv_stage, m, (0,)), 32))
                items.append(('pw', functools.partial(pv_stage, m, (1,)), 32))
                items.append(('pw', functools.partial(pv_stage, m, (2,)), 32))
            if pend and n >= pend[0][0]:
                items.append(pend.pop(0)[1])
            if m % NG == NG - 1:
                pend.append((n + cfg['WOD'], ('wo', functools.partial(wo_stage, m // NG), 800, m // NG)))
    items += [w[1] for w in pend]
    return items


def _c_items(R, base, du, par, hbuf=0, free=False):
    h1_ref, hn_ref, g_ref = R.h1[hbuf], R.hn[hbuf], R.g[par]
    w0, w1 = (None, None) if free else (('wo', 0), ('wo', 1))

    def f1(c):
        u = jnp.dot(_as_bf16(hn_ref[...]), _as_bf16(R.w1[:, 128 * c:128 * c + 128]),
                    preferred_element_type=f32)
        u = u + R.b1[128 * c:128 * c + 128].astype(f32).reshape(1, 128)
        g_ref[:, 128 * c:128 * c + 128] = _words(_gelu(u))

    def f2(m, n):
        g = _as_bf16(g_ref[64 * m:64 * m + 64, :])
        y = jnp.dot(g, _as_bf16(R.w2[:, 128 * n:128 * n + 128]), preferred_element_type=f32)
        y = y + R.b2[128 * n:128 * n + 128].astype(f32).reshape(1, 128)
        R.o[pl.ds(base['xrow'] + du * TQ + 128 * m, 128), 128 * n:128 * n + 128] = (
            h1_ref[128 * m:128 * m + 128, 128 * n:128 * n + 128] + y).astype(bf16)

    return dict(
        f1=[('f1', functools.partial(f1, c), 320, None, w0) for c in range(F // 128)],
        f2a=[('f2', functools.partial(f2, 0, n), 384, None, w0) for n in range(D // 128)],
        f2b=[('f2', functools.partial(f2, 1, n), 384, None, w1) for n in range(D // 128)],
    )


def _merge(main, fill, cfg):
    fill = [it if len(it) == 5 else it + (None, None) for it in fill]
    t1, t2 = cfg['TAIL']
    t2 = min(t2, len(fill))
    t1 = min(t1, len(fill) - t2)
    nmid = len(fill) - t1 - t2
    first = cfg['START']
    tot_f = sum(it[2] for it in main[first:-1])
    tot_b = sum(it[2] for it in fill[:nmid])
    out, done = [], set()
    todo = list(range(len(fill)))
    acc = [0, 0]

    def emit(k):
        todo.remove(k)
        out.append(fill[k])
        acc[1] += fill[k][2]

    for k, it in enumerate(main):
        tag = (it[0], it[3]) if len(it) > 3 else None
        if k == len(main) - 1:
            for f in [f for f in todo if f < nmid + t1]:
                emit(f)
        elif k >= first and it[0] in cfg['INS']:
            while True:
                cand = [f for f in todo if f < nmid and (fill[f][3] is None or fill[f][3] in done)]
                if not cand or acc[1] + fill[cand[0]][2] * cfg['BIAS'] > acc[0] * tot_b / tot_f:
                    break
                emit(cand[0])
        if tag is not None:
            for f in [f for f in todo if fill[f][4] == tag]:
                emit(f)
        if k >= first:
            acc[0] += it[2]
        out.append(it)
        done.add(tag)
    for f in list(todo):
        emit(f)
    return out


def _phase(R, base, z, cfg, a=None, b=None, c=None, akw={}, bkw={}, ckw={}, extra=()):
    parts = {}
    if a is not None:
        parts.update(_a_items(R, None, base, a[0], a[1], cfg, **akw))
    if c is not None:
        parts.update(_c_items(R, base, c[0], c[1], **ckw))
    fill = list(extra)
    for key in cfg['ORDER'].split(','):
        fill += parts.get(key, [])
    pre = parts.get('ln', [])
    if b is None:
        return pre + fill
    return pre + _merge(_b_items(R, base, b[0], b[1], cfg, z, **bkw), fill, cfg)


def _kernel(x_hbm, wqkv_hbm, wo_hbm, w1_hbm, b1_hbm, w2_hbm, b2_hbm, o_hbm,
            x_ref, o_ref, kg_ref, vt_ref, wvt_ref, wq_ref, wk_ref, wv_ref, wo_ref, w1_ref, w2_ref,
            p0_ref, p1_ref, p2_ref, z_ref,
            xn0, xn1, xs0, xs1, g0, g1, q_ref, s_ref, ot_ref, h1_ref, hn_ref,
            qa_ref, h1a_ref, hna_ref, b1_ref, b2_ref,
            sem, xsem, osem, *, cfg):
    i = pl.program_id(0)
    R = _Refs()
    R.x, R.o, R.kg, R.vt, R.wvt = x_ref, o_ref, kg_ref, vt_ref, wvt_ref
    R.wq, R.wk, R.wo, R.w1, R.w2, R.b1, R.b2 = wq_ref, wk_ref, wo_ref, w1_ref, w2_ref, b1_ref, b2_ref
    R.p = (p0_ref, p1_ref, p2_ref)
    R.xn, R.xs, R.g = (xn0, xn1), (xs0, xs1), (g0, g1)
    R.q, R.s, R.ot = q_ref, s_ref, ot_ref
    R.h1, R.hn = (h1_ref, h1a_ref), (hn_ref, hna_ref)
    only = cfg['ONLY']
    gcfg = cfg

    def rcfg(name):
        c = dict(gcfg)
        c.update(gcfg.get(name) or {})
        return c

    KS, QS = cfg['KS'], cfg['QS']
    specs = dict(
        ka=(wqkv_hbm, D, wk_ref, 0, 128 * KS), kb=(wqkv_hbm, D, wk_ref, 128 * KS, D - 128 * KS),
        qa=(wqkv_hbm, 0, wq_ref, 0, 128 * QS), qb=(wqkv_hbm, 0, wq_ref, 128 * QS, D - 128 * QS),
        v=(wqkv_hbm, 2 * D, wv_ref, 0, D), o=(wo_hbm, 0, wo_ref, 0, D),
        w1=(w1_hbm, 0, w1_ref, 0, F), w2=(w2_hbm, 0, w2_ref, 0, D))
    copies = {}
    for n, (name, (src, c0, dst, d0, nc)) in enumerate(specs.items()):
        if nc > 0:
            copies[name] = pltpu.make_async_copy(
                src.bitcast(i32).at[:, pl.ds(c0 + d0, nc)], dst.at[:, pl.ds(d0, nc)], sem.at[n])

    copies['b1'] = pltpu.make_async_copy(b1_hbm, b1_ref, sem.at[8])
    copies['b2'] = pltpu.make_async_copy(b2_hbm, b2_ref, sem.at[9])

    def xcopy(b):
        h = TQ // 2
        return pltpu.make_async_copy(x_hbm.bitcast(i32).at[0, pl.ds(b * h, h), :],
                                     x_ref.at[pl.ds(b * h, h), :], xsem.at[b])

    def ocopy(b):
        return pltpu.make_async_copy(o_ref.at[pl.ds(b * TQ, TQ), :],
                                     o_hbm.at[0, pl.ds(b * TQ, TQ), :], osem.at[b])

    def static_base(u):
        return dict(krow=u * (TQ // 2), xrow=u * TQ, kb=u * NB)

    @pl.when(i == 0)
    def _first():
        if only not in (None, 'first'):
            return
        cfg = rcfg('first')
        plan = cfg['PLAN']

        def go(p):
            for name in plan.get(p, '').split():
                if name[0] == 'x':
                    xcopy(int(name[1:])).start()
                elif name in copies:
                    copies[name].start()

        def wait(name):
            if name in copies:
                copies[name].wait()
            go(name)

        go('start')
        z_ref[0] = 0
        lane1 = lax.broadcasted_iota(i32, (W // 2, 128), 1)
        for g in range(NG):
            sp = (80 * g + 80) % 128
            kg_ref[g, 0:W // 2, :] = jnp.where(lane1 == sp, ONE_WORD, 0).astype(i32)
        vt_ref[0:2] = jnp.zeros((2, H * 16, 128), i32)
        xcopy(0).wait()
        go('x0')
        base = static_base(0)
        a0 = _a_items(R, None, base, 0, 0, cfg, q_ref=qa_ref)
        a0['ln'][0][1]()
        wait('ka')
        for it in a0['k'][:KS]:
            it[1]()
        wait('kb')
        for it in a0['k'][KS:]:
            it[1]()
        wait('qa')
        for it in a0['q'][:QS]:
            it[1]()
        wait('qb')
        for it in a0['q'][QS:]:
            it[1]()
        z = z_ref[0]
        items = _phase(R, base, z, cfg, a=(1, 1), b=(0, 0), akw=dict(free=True),
                       bkw=dict(q_ref=qa_ref))

        def vwait():
            xcopy(1).wait()
            wait('v')
            if cfg['OEARLY']:
                wait('o')
            wvt_ref[...] = _words(_as_bf16(wv_ref[...]).astype(f32).T)

        ln1, items = items[0], items[1:]
        lead = [it for it in items if it[0] in ('qk', 'sm')][:2 * cfg['WV']]
        items = [it for it in items if not any(it is l for l in lead)]
        k = next(n for n, it in enumerate(items) if it[0] == 'pv')
        items = lead + [('w', vwait), ln1] + items[:k] + a0['v'] + items[k:]
        k = next(n for n, it in enumerate(items) if it[0] == 'wo') - cfg['WOW']
        for n, it in enumerate(items):
            if n == k and not cfg['OEARLY']:
                wait('o')
            it[1]()
        go('end')
        wait('w1')
        wait('w2')
        wait('b1')
        wait('b2')

    @pl.when((i > 0) & (i < NU - 1))
    def _mid():
        if only not in (None, 'mid'):
            return
        cfg = rcfg('mid')
        xcopy(i + 1).wait()
        base = dict(krow=pl.multiple_of((i - 1) * (TQ // 2), TQ // 2),
                    xrow=pl.multiple_of((i - 1) * TQ, TQ), kb=(i - 1) * NB)
        z = z_ref[0]
        for it in _phase(R, base, z, cfg, a=(2, 0), b=(1, 0), c=(0, 0)):
            it[1]()
        ocopy(i - 1).start()

    @pl.when(i == NU - 1)
    def _last():
        if only not in (None, 'last'):
            return
        cfg = rcfg('last')
        base = static_base(NU - 2)
        z = z_ref[0]
        for it in _phase(R, base, z, cfg, b=(1, 0), c=(0, 0), bkw=dict(hbuf=1), ckw=dict(free=True)):
            it[1]()
        ocopy(NU - 2).start()
        r0 = (NU - 1) * TQ
        pieces = {16: (r0, 128, 0, D), 16 + cfg['OSPL']: (r0 + 128, 128, 0, 128 * cfg['OSPL']),
                  21: (r0 + 128, 128, 128 * cfg['OSPL'], D - 128 * cfg['OSPL'])}
        tail = []
        for n, it in enumerate(_phase(R, base, z, cfg, c=(1, 1), ckw=dict(hbuf=1))):
            it[1]()
            if n in pieces:
                r, nr, c, nc = pieces[n]
                cp = pltpu.make_async_copy(o_ref.at[pl.ds(r, nr), pl.ds(c, nc)],
                                           o_hbm.at[0, pl.ds(r, nr), pl.ds(c, nc)],
                                           osem.at[NU - 1 + len(tail)])
                cp.start()
                tail.append(cp)
        for b in range(NU - 1):
            ocopy(b).wait()
        for cp in tail:
            cp.wait()


def make(**kw):
    cfg = dict(DEFAULT_CFG)
    cfg.update(kw)

    @jax.jit
    def fn(A_x, A_wqkv, A_wo, B_x, B_w1, B_b1, B_w2, B_b2):
        del B_x
        hbm = pl.BlockSpec(memory_space=pl.ANY)
        two = lambda shape, dt: [pltpu.VMEM(shape, dt)] * 2
        return pl.pallas_call(
            functools.partial(_kernel, cfg=cfg),
            grid=(NU,),
            in_specs=[
                hbm, hbm, hbm, hbm, hbm, hbm, hbm,
            ],
            out_specs=hbm,
            out_shape=jax.ShapeDtypeStruct((1, S, D), bf16),
            scratch_shapes=[
                pltpu.VMEM((S // 2, D), i32),
                pltpu.VMEM((S, D), bf16),
                pltpu.VMEM((NG, (S + W) // 2, 128), i32),
                pltpu.VMEM((S // 128 + 2, H * 16, 128), i32),
                pltpu.VMEM((D // 2, D), i32),
                pltpu.VMEM((D // 2, D), i32),
                pltpu.VMEM((D // 2, D), i32),
                pltpu.VMEM((D // 2, D), i32),
                pltpu.VMEM((D // 2, D), i32),
                pltpu.VMEM((D // 2, F), i32),
                pltpu.VMEM((F // 2, D), i32),
                pltpu.VMEM((5, 128, 128), i32),
                pltpu.VMEM((5, 128, 128), i32),
                pltpu.VMEM((5, 128, 128), i32),
                pltpu.SMEM((1,), i32),
            ] + two((TQ // 2, D), i32) + two((TQ // 2, D), i32) + two((TQ // 2, F), i32) + [
                pltpu.VMEM((NG, TQ // 2, 128), i32),
                pltpu.VMEM((TQ // 4, 256, 128), f32),
                pltpu.VMEM((NB, D, 128), f32),
                pltpu.VMEM((TQ, D), f32),
                pltpu.VMEM((TQ // 2, D), i32),
                pltpu.VMEM((NG, TQ // 2, 128), i32),
                pltpu.VMEM((TQ, D), f32),
                pltpu.VMEM((TQ // 2, D), i32),
                pltpu.VMEM((F,), bf16),
                pltpu.VMEM((D,), bf16),
                pltpu.SemaphoreType.DMA((10,)),
                pltpu.SemaphoreType.DMA((NU,)),
                pltpu.SemaphoreType.DMA((NU + 2,)),
            ],
            compiler_params=pltpu.CompilerParams(
                dimension_semantics=("arbitrary",),
                vmem_limit_bytes=100 * 2**20),
        )(A_x, A_wqkv, A_wo, B_w1, B_b1, B_w2, B_b2)
    return fn


pallas_sequential_preLN__sliding_block__dense_activation_gelu__prompt_kernel = make()
```

```python
import functools
import math

import jax
import jax.numpy as jnp
from jax import lax
import jax.experimental.pallas as pl
import jax.experimental.pallas.tpu as pltpu

S = 2048
D = 640
F = 1536
H = 32
DH = 20
W = 256
NG = 8
TQ = 256
NB = TQ // 128
NU = S // TQ
EPS = 1e-5
QSCALE = (DH ** -0.5) * math.log2(math.e)
NEG_WORD = -243207808
ONE_WORD = 0x3F803F80
KS = 2
SS = 16
SD = 2

f32 = jnp.float32
bf16 = jnp.bfloat16
i32 = jnp.int32

CFG_FIRST = dict(DEPTH=2, REL=((0, 0), (0, 96), (0, 168)), WOD=3, INS=('pv', 'qk'), TAIL=(0, 3),
                 START=5, VCH=4, ORDER='f1,f2a,f2b,v,k,q', BIAS=1.5, MINT=4)
CFG_MID = dict(DEPTH=2, REL=((0, 48), (0, 144), (0, 200)), WOD=4, INS=('pv', 'qk'), TAIL=(1, 4),
               START=2, VCH=8, ORDER='f1,f2a,f2b,k,v,q', BIAS=1.0, MINT=4)
CFG_LAST = dict(DEPTH=1, REL=((0, 24), (0, 120), (0, 240)), WOD=3, INS=('pv',), TAIL=(1, 2),
                START=3, VCH=8, ORDER='f1,f2a,f2b,k,v,q', BIAS=0.0, MINT=2)
DMA_PLAN = dict(start='x0 x1 ka kb', x0='q', ka='v o', kb='w1 w2 x2 b1 b2 x3 x4 x5 x6 x7')


def _ln(x):
    m = jnp.mean(x, axis=-1, keepdims=True)
    xc = x - m
    v = jnp.mean(xc * xc, axis=-1, keepdims=True)
    return xc * lax.rsqrt(v + EPS)


def _gelu(x):
    c = math.sqrt(2.0 / math.pi)
    return 0.5 * x * (1.0 + jnp.tanh(c * (x + 0.044715 * (x * x * x))))


def _pack_pairs(a, odd, round_up):
    u = pltpu.bitcast(a, i32)
    if round_up:
        u = u + 0x8000
    rows = []
    for r in range(0, a.shape[0], 16):
        cols = []
        for c in range(0, a.shape[1], 128):
            lo = lax.shift_right_logical(u[r:r + 8, c:c + 128], 16)
            w = jnp.where(odd, pltpu.bitcast(u[r + 8:r + 16, c:c + 128], bf16),
                          pltpu.bitcast(lo, bf16))
            cols.append(pltpu.bitcast(w, i32))
        rows.append(cols[0] if len(cols) == 1 else jnp.concatenate(cols, axis=1))
    return rows[0] if len(rows) == 1 else jnp.concatenate(rows, axis=0)


def _odd_rows():
    return (lax.broadcasted_iota(i32, (16, 128), 0) & 1) == 1


def _words(a):
    return pltpu.bitcast(a.astype(bf16), i32)


def _as_bf16(w):
    return pltpu.bitcast(w, bf16)


def _group_tile(tiles, g, lane, zero_rest):
    lo = 80 * g
    t, off = lo // 128, lo % 128
    if off + 80 <= 128:
        if zero_rest:
            return jnp.where((lane >= off) & (lane < off + 80), tiles[t], 0)
        return tiles[t]
    e = off + 80 - 128
    if zero_rest:
        return jnp.where(lane < e, tiles[t + 1], jnp.where(lane >= off, tiles[t], 0))
    return jnp.where(lane < e, tiles[t + 1], tiles[t])


def _groups_ready(t):
    return [g for g in range(NG) if (80 * g + 79) // 128 == t]


def _sel(m, t, f_):
    if t is None and f_ is None:
        return None
    if t is None:
        t = 0
    if f_ is None:
        f_ = 0
    return jnp.where(m, t, f_)


class _Refs:
    pass


def _a_items(R, base, du, par, cfg, q_ref=None, free=False):
    st = {}
    xn_ref, xs_ref = R.xn[par], R.xs[par]
    q_ref = R.q if q_ref is None else q_ref
    row0 = base['krow'] + du * (TQ // 2)

    def ln1():
        x = R.x[pl.ds(base['xrow'] + du * TQ, TQ), :].astype(f32)
        xnf = _ln(x)
        xn_ref[...] = _words(xnf)
        xs_ref[...] = _pack_pairs(xnf, _odd_rows(), True)

    def kproj(t):
        k = jnp.dot(_as_bf16(xn_ref[...]), R.wk[:, 128 * t:128 * t + 128],
                    preferred_element_type=f32)
        st[('k', t)] = _words(k)
        lane = lax.broadcasted_iota(i32, (TQ // 2, 128), 1)
        tiles = {tt: st[('k', tt)] for tt in range(t + 1)}
        for g in _groups_ready(t):
            R.kg[g, pl.ds(row0 + W // 2, TQ // 2), :] = _group_tile(tiles, g, lane, True)

    def qproj(t):
        q = jnp.dot(_as_bf16(xn_ref[...]), R.wq[:, 128 * t:128 * t + 128],
                    preferred_element_type=f32) * QSCALE
        st[('q', t)] = _words(q)
        lane = lax.broadcasted_iota(i32, (TQ // 2, 128), 1)
        tiles = {tt: st[('q', tt)] for tt in range(t + 1)}
        for g in _groups_ready(t):
            q_ref[g] = _group_tile(tiles, g, lane, False)

    def vproj(c):
        gpc = NG // cfg['VCH']
        m0 = 80 * gpc * c
        vt = lax.dot_general(_as_bf16(R.wvt[m0 // 2:m0 // 2 + 40 * gpc, :]), _as_bf16(xs_ref[...]),
                             (((1,), (1,)), ((), ())), preferred_element_type=f32)
        vtw = _words(vt)
        sub8 = lax.broadcasted_iota(i32, (8, TQ), 0)
        pieces = []
        for gg in range(gpc):
            for hh in range(4):
                w0 = 40 * gg + 8 * hh
                a = vtw[w0:w0 + 8]
                b = vtw[w0 + 8:w0 + 16]
                if hh < 2:
                    b = jnp.where(sub8 >= 4, ONE_WORD, b)
                else:
                    a = jnp.where(sub8 < 4, ONE_WORD, a)
                pieces += [a, b]
        vtp = jnp.concatenate(pieces, axis=0)
        for nb in range(NB):
            R.vt[base['kb'] + du * NB + nb + 2, 64 * gpc * c:64 * gpc * (c + 1), :] = (
                vtp[:, 128 * nb:128 * nb + 128])

    return dict(
        ln=[('ln1', ln1, 0)],
        k=[('k', functools.partial(kproj, t), 320) for t in range(5)],
        q=[('q', functools.partial(qproj, t), 320,
            None if free else ('qk', NG + max(_groups_ready(t))), None) for t in range(5)],
        v=[('v', functools.partial(vproj, c), 1600 // cfg['VCH']) for c in range(cfg['VCH'])],
    )


def _b_items(R, base, du, cfg, z, q_ref=None, hbuf=0):
    st = {}
    s_ref, ot_ref = R.s, R.ot
    q_ref = R.q if q_ref is None else q_ref
    h1_ref, hn_ref = R.h1[hbuf], R.hn[hbuf]
    row0 = base['krow'] + du * (TQ // 2)
    DEPTH, MINT = cfg['DEPTH'], cfg['MINT']

    lane16 = lax.broadcasted_iota(i32, (16, 128), 1)
    r16 = lax.broadcasted_iota(i32, (16, 128), 0)
    cw = lane16 & 31
    odd16 = _odd_rows()
    tri0 = r16 > cw
    tri1 = r16 + 16 > cw
    rw = (r16 & 7) + 2 * (r16 & 8)
    m_old = (jnp.where(rw > cw, 0xFFFF, 0) | jnp.where(rw + 8 > cw, -65536, 0)).astype(i32)
    m_new = ~m_old
    s_odd = (lane16 & 32) != 0
    s_hi = (lane16 & 64) != 0
    sub8b = lax.broadcasted_iota(i32, (8, 128), 0) < 4

    def qk_stage(n):
        nb, g = n // NG, n % NG
        off = (80 * g) % 128
        rel = (lane16 - off) & 127
        cneg = jnp.where(rel == 80, NEG_WORD, 0).astype(i32)
        hmask = [(rel >= 20 * hh) & (rel < 20 * hh + 20) for hh in range(4)]
        for j in range(4):
            jj = 4 * nb + j
            qs = q_ref[g, 16 * jj:16 * jj + 16, :]
            bmat = _as_bf16(jnp.concatenate(
                [jnp.where(hmask[s ^ j], qs, cneg) for s in range(4)], axis=0))
            kw = R.kg[g, pl.ds(row0 + 16 * jj, 144), :]
            kwin = _as_bf16(jnp.concatenate(
                [kw[16:128], kw[0:8], kw[128:136], kw[8:16], kw[136:144]], axis=0))
            s_t = lax.dot_general(kwin, bmat, (((1,), (1,)), ((), ())),
                                  preferred_element_type=f32)
            slot = n * 4 + j
            e0 = jnp.where(tri0, s_t[224:240], s_t[240:256])
            e1 = jnp.where(tri1, s_t[256:272], s_t[272:288])
            sm = jnp.concatenate([s_t[0:224], e0, e1], axis=0)
            m = None
            for r in range(0, 256, 8):
                v = sm[r:r + 8]
                if m is None:
                    m = v
                    s_ref[slot, r:r + 8, :] = v
                else:
                    m = jnp.maximum(m, v)
                    tie = (r // 8) % MINT == MINT - 1
                    s_ref[slot, r:r + 8, :] = jnp.minimum(v, m) if tie else v
            st[('mx', n, j)] = jnp.max(m, axis=0, keepdims=True)
            st[('st', n, j)] = s_t

    def sm_stage(n):
        for j in range(4):
            slot = n * 4 + j
            mx = jnp.broadcast_to(st.pop(('mx', n, j)), (8, 128))
            hist = []
            for r in range(0, 256, SS):
                if len(hist) >= SD:
                    mx = jnp.maximum(mx, hist[-SD] - 3e38)
                p = jnp.exp2(s_ref[slot, r:r + SS, :] - jnp.concatenate([mx] * (SS // 8), axis=0))
                hist.append(p[SS - 8:SS])
                R.p[n % 3][j, r // 2:(r + SS) // 2, :] = _pack_pairs(p, odd16, False)

    def pv_stage(n):
        nb, g = n // NG, n % NG
        p_ref = R.p[n % 3]
        kb = base['kb'] + du * NB + nb
        acc = [None] * 4
        for t in range(3):
            spec = cfg['REL'][t]
            if spec is not None and ('st', n + DEPTH, spec[0]) in st:
                s_t = st[('st', n + DEPTH, spec[0])]
                p_ref[4, 8 * t:8 * t + 8, :] = pltpu.bitcast(s_t[spec[1]:spec[1] + 8], i32)

            def blk(j, b):
                if b < 0 or b > 8:
                    return None
                if b == 0:
                    return p_ref[z + j, 112:128, :] & m_old
                if b == 8:
                    return p_ref[z + j, 112:128, :] & m_new
                return p_ref[z + j, 16 * (b - 1):16 * b, :]

            wrows = [[], [], [], []]
            for a in range(4 * t, 4 * t + 4):
                X = [blk(j, a - j) for j in range(4)]
                Y = [_sel(s_odd, X[1], X[0]), _sel(s_odd, X[0], X[1]),
                     _sel(s_odd, X[3], X[2]), _sel(s_odd, X[2], X[3])]
                Z = [_sel(s_hi, Y[2], Y[0]), _sel(s_hi, Y[3], Y[1]),
                     _sel(s_hi, Y[0], Y[2]), _sel(s_hi, Y[1], Y[3])]
                for hh in range(4):
                    wrows[hh].append(Z[hh])
            for hh in range(4):
                h = 4 * g + hh
                wm = _as_bf16(jnp.concatenate(wrows[hh], axis=0))
                vl = _as_bf16(R.vt[kb + t, 16 * h:16 * h + 16, :])
                ot = jnp.dot(vl, wm, preferred_element_type=f32)
                acc[hh] = ot if acc[hh] is None else acc[hh] + ot
        on = []
        for hh in range(4):
            ot = acc[hh]
            den = ot[24:32] if hh < 2 else ot[0:8]
            r = 1.0 / den
            on.append([ot[8 * t:8 * t + 8] * r for t in range(4)])
        ot_ref[nb, 80 * g:80 * g + 80, :] = jnp.concatenate(
            [on[0][0], on[0][1], jnp.where(sub8b, on[0][2], on[1][0]),
             on[1][1], on[1][2], on[2][1], on[2][2],
             jnp.where(sub8b, on[2][3], on[3][1]), on[3][2], on[3][3]], axis=0)

    def wo_stage(nb):
        t = ot_ref[nb].T
        lane640 = lax.broadcasted_iota(i32, (32, D), 1)
        hid = lane640 // DH
        b0 = (hid & 1) != 0
        b1 = (hid & 2) != 0
        X = [t[32 * j:32 * j + 32] for j in range(4)]
        Y = [jnp.where(b0, X[j ^ 1], X[j]) for j in range(4)]
        Z = [jnp.where(b1, Y[j ^ 2], Y[j]) for j in range(4)]
        o = jnp.concatenate(Z, axis=0).astype(bf16)
        x = R.x[pl.ds(base['xrow'] + du * TQ + 128 * nb, 128), :].astype(f32)
        h1 = x + jnp.dot(o, R.wo[...], preferred_element_type=f32)
        h1_ref[128 * nb:128 * nb + 128, :] = h1
        hn_ref[64 * nb:64 * nb + 64, :] = _words(_ln(h1))

    items = []
    NA = NB * NG
    pend = []
    for n in range(NA + DEPTH):
        if n < NA:
            items.append(('qk', functools.partial(qk_stage, n), 288, n))
            items.append(('sm', functools.partial(sm_stage, n), 0))
        m = n - DEPTH
        if m >= 0:
            items.append(('pv', functools.partial(pv_stage, m), 96))
            if pend and n >= pend[0][0]:
                items.append(pend.pop(0)[1])
            if m % NG == NG - 1:
                pend.append((n + cfg['WOD'],
                             ('wo', functools.partial(wo_stage, m // NG), 800, m // NG)))
    items += [w[1] for w in pend]
    return items


def _c_items(R, base, du, par, hbuf=0, free=False):
    h1_ref, hn_ref, g_ref = R.h1[hbuf], R.hn[hbuf], R.g[par]
    w0, w1 = (None, None) if free else (('wo', 0), ('wo', 1))

    def f1(c):
        u = jnp.dot(_as_bf16(hn_ref[...]), R.w1[:, 128 * c:128 * c + 128],
                    preferred_element_type=f32)
        u = u + R.b1[128 * c:128 * c + 128].astype(f32).reshape(1, 128)
        g_ref[:, 128 * c:128 * c + 128] = _words(_gelu(u))

    def f2(m, n):
        g = _as_bf16(g_ref[64 * m:64 * m + 64, :])
        y = jnp.dot(g, R.w2[:, 128 * n:128 * n + 128], preferred_element_type=f32)
        y = y + R.b2[128 * n:128 * n + 128].astype(f32).reshape(1, 128)
        R.o[pl.ds(base['xrow'] + du * TQ + 128 * m, 128), 128 * n:128 * n + 128] = (
            h1_ref[128 * m:128 * m + 128, 128 * n:128 * n + 128] + y).astype(bf16)

    return dict(
        f1=[('f1', functools.partial(f1, c), 320, None, w0) for c in range(F // 128)],
        f2a=[('f2', functools.partial(f2, 0, n), 384, None, w0) for n in range(D // 128)],
        f2b=[('f2', functools.partial(f2, 1, n), 384, None, w1) for n in range(D // 128)],
    )


def _merge(main, fill, cfg):
    fill = [it if len(it) == 5 else it + (None, None) for it in fill]
    t1, t2 = cfg['TAIL']
    t2 = min(t2, len(fill))
    t1 = min(t1, len(fill) - t2)
    nmid = len(fill) - t1 - t2
    first = cfg['START']
    tot_f = sum(it[2] for it in main[first:-1])
    tot_b = sum(it[2] for it in fill[:nmid])
    out, done = [], set()
    todo = list(range(len(fill)))
    acc = [0, 0]

    def emit(k):
        todo.remove(k)
        out.append(fill[k])
        acc[1] += fill[k][2]

    for k, it in enumerate(main):
        tag = (it[0], it[3]) if len(it) > 3 else None
        if k == len(main) - 1:
            for f in [f for f in todo if f < nmid + t1]:
                emit(f)
        elif k >= first and it[0] in cfg['INS']:
            while True:
                cand = [f for f in todo if f < nmid and (fill[f][3] is None or fill[f][3] in done)]
                if not cand or acc[1] + fill[cand[0]][2] * cfg['BIAS'] > acc[0] * tot_b / tot_f:
                    break
                emit(cand[0])
        if tag is not None:
            for f in [f for f in todo if fill[f][4] == tag]:
                emit(f)
        if k >= first:
            acc[0] += it[2]
        out.append(it)
        done.add(tag)
    for f in list(todo):
        emit(f)
    return out


def _phase(parts, main, cfg):
    fill = []
    for key in cfg['ORDER'].split(','):
        fill += parts.get(key, [])
    pre = parts.get('ln', [])
    if main is None:
        return pre + fill
    return pre + _merge(main, fill, cfg)


def _run(items):
    for it in items:
        it[1]()


def _kernel(x_hbm, wqkv_hbm, wo_hbm, w1_hbm, b1_hbm, w2_hbm, b2_hbm, o_hbm,
            x_ref, o_ref, kg_ref, vt_ref, wvt_ref, wq_ref, wk_ref, wv_ref, wo_ref, w1_ref, w2_ref,
            p0_ref, p1_ref, p2_ref, z_ref,
            xn0, xn1, xs0, xs1, g0, g1, q_ref, s_ref, ot_ref, h1_ref, hn_ref,
            qa_ref, h1a_ref, hna_ref, b1_ref, b2_ref,
            sem, xsem, osem):
    i = pl.program_id(0)
    R = _Refs()
    R.x, R.o, R.kg, R.vt, R.wvt = x_ref, o_ref, kg_ref, vt_ref, wvt_ref
    R.wq, R.wk, R.wo, R.w1, R.w2, R.b1, R.b2 = wq_ref, wk_ref, wo_ref, w1_ref, w2_ref, b1_ref, b2_ref
    R.p = (p0_ref, p1_ref, p2_ref)
    R.xn, R.xs, R.g = (xn0, xn1), (xs0, xs1), (g0, g1)
    R.q, R.s, R.ot = q_ref, s_ref, ot_ref
    R.h1, R.hn = (h1_ref, h1a_ref), (hn_ref, hna_ref)

    def xcopy(b):
        return pltpu.make_async_copy(x_hbm.at[0, pl.ds(b * TQ, TQ), :],
                                     x_ref.at[pl.ds(b * TQ, TQ), :], xsem.at[b])

    def ocopy(b):
        return pltpu.make_async_copy(o_ref.at[pl.ds(b * TQ, TQ), :],
                                     o_hbm.at[0, pl.ds(b * TQ, TQ), :], osem.at[b])

    def static_base(u):
        return dict(krow=u * (TQ // 2), xrow=u * TQ, kb=u * NB)

    def opaque_zero():
        return jnp.clip(z_ref[0], 0, 1)

    @pl.when(i == 0)
    def _first():
        cfg = CFG_FIRST
        specs = dict(
            ka=(wqkv_hbm, D, wk_ref, 0, 128 * KS), kb=(wqkv_hbm, D, wk_ref, 128 * KS, D - 128 * KS),
            q=(wqkv_hbm, 0, wq_ref, 0, D), v=(wqkv_hbm, 2 * D, wv_ref, 0, D),
            o=(wo_hbm, 0, wo_ref, 0, D), w1=(w1_hbm, 0, w1_ref, 0, F), w2=(w2_hbm, 0, w2_ref, 0, D))
        copies = {}
        for n, (name, (src, c0, dst, d0, nc)) in enumerate(specs.items()):
            copies[name] = pltpu.make_async_copy(
                src.at[:, pl.ds(c0 + d0, nc)], dst.at[:, pl.ds(d0, nc)], sem.at[n])
        copies['b1'] = pltpu.make_async_copy(b1_hbm, b1_ref, sem.at[7])
        copies['b2'] = pltpu.make_async_copy(b2_hbm, b2_ref, sem.at[8])

        def go(p):
            for name in DMA_PLAN.get(p, '').split():
                if name[0] == 'x':
                    xcopy(int(name[1:])).start()
                else:
                    copies[name].start()

        def wait(name):
            copies[name].wait()
            go(name)

        go('start')
        z_ref[0] = 0
        lane1 = lax.broadcasted_iota(i32, (W // 2, 128), 1)
        for g in range(NG):
            sp = (80 * g + 80) % 128
            kg_ref[g, 0:W // 2, :] = jnp.where(lane1 == sp, ONE_WORD, 0).astype(i32)
        vt_ref[0:2] = jnp.zeros((2, H * 16, 128), i32)
        for p_ref in R.p:
            p_ref[...] = jnp.zeros(p_ref.shape, i32)
        xcopy(0).wait()
        go('x0')
        base = static_base(0)
        a0 = _a_items(R, base, 0, 0, cfg, q_ref=qa_ref)
        a1 = _a_items(R, base, 1, 1, cfg, free=True)
        _run(a0['ln'])
        xcopy(1).wait()
        wait('ka')
        _run(a0['k'][:KS] + a1['ln'] + a1['k'][:KS])
        wait('kb')
        _run(a0['k'][KS:] + a1['k'][KS:])
        wait('q')
        _run(a0['q'])
        items = _phase(dict(q=a1['q'], v=a1['v']),
                       _b_items(R, base, 0, cfg, opaque_zero(), q_ref=qa_ref), cfg)
        lead = [it for it in items if it[0] in ('qk', 'sm')][:4]
        items = [it for it in items if not any(it is l for l in lead)]
        k = next(n for n, it in enumerate(items) if it[0] == 'pv')
        _run(lead)
        wait('v')
        wait('o')
        wvt_ref[...] = _words(wv_ref[...].astype(f32).T)
        _run(items[:k] + a0['v'] + items[k:])
        wait('w1')
        wait('w2')
        wait('b1')
        wait('b2')

    @pl.when((i > 0) & (i < NU - 1))
    def _mid():
        cfg = CFG_MID
        xcopy(i + 1).wait()
        base = dict(krow=pl.multiple_of((i - 1) * (TQ // 2), TQ // 2),
                    xrow=pl.multiple_of((i - 1) * TQ, TQ), kb=(i - 1) * NB)
        z = opaque_zero()
        parts = _a_items(R, base, 2, 0, cfg)
        parts.update(_c_items(R, base, 0, 0))
        _run(_phase(parts, _b_items(R, base, 1, cfg, z), cfg))
        ocopy(i - 1).start()

    @pl.when(i == NU - 1)
    def _last():
        cfg = CFG_LAST
        base = static_base(NU - 2)
        z = opaque_zero()
        _run(_phase(_c_items(R, base, 0, 0, free=True), _b_items(R, base, 1, cfg, z, hbuf=1), cfg))
        ocopy(NU - 2).start()
        r0 = (NU - 1) * TQ
        pieces = {16: (r0, 0, D), 20: (r0 + 128, 0, 512), 21: (r0 + 128, 512, D - 512)}
        tail = []
        for n, it in enumerate(_phase(_c_items(R, base, 1, 1, hbuf=1), None, cfg)):
            it[1]()
            if n in pieces:
                r, c, nc = pieces[n]
                cp = pltpu.make_async_copy(o_ref.at[pl.ds(r, 128), pl.ds(c, nc)],
                                           o_hbm.at[0, pl.ds(r, 128), pl.ds(c, nc)],
                                           osem.at[NU - 1 + len(tail)])
                cp.start()
                tail.append(cp)
        for b in range(NU - 1):
            ocopy(b).wait()
        for cp in tail:
            cp.wait()


@jax.jit
def pallas_sequential_preLN__sliding_block__dense_activation_gelu__prompt_kernel(
    A_x: jax.Array,
    A_wqkv: jax.Array,
    A_wo: jax.Array,
    B_x: jax.Array,
    B_w1: jax.Array,
    B_b1: jax.Array,
    B_w2: jax.Array,
    B_b2: jax.Array,
):
    del B_x
    hbm = pl.BlockSpec(memory_space=pl.ANY)
    return pl.pallas_call(
        _kernel,
        grid=(NU,),
        in_specs=[hbm] * 7,
        out_specs=hbm,
        out_shape=jax.ShapeDtypeStruct((1, S, D), bf16),
        scratch_shapes=[
            pltpu.VMEM((S, D), bf16),
            pltpu.VMEM((S, D), bf16),
            pltpu.VMEM((NG, (S + W) // 2, 128), i32),
            pltpu.VMEM((S // 128 + 2, H * 16, 128), i32),
            pltpu.VMEM((D // 2, D), i32),
            pltpu.VMEM((D, D), bf16),
            pltpu.VMEM((D, D), bf16),
            pltpu.VMEM((D, D), bf16),
            pltpu.VMEM((D, D), bf16),
            pltpu.VMEM((D, F), bf16),
            pltpu.VMEM((F, D), bf16),
            pltpu.VMEM((5, 128, 128), i32),
            pltpu.VMEM((5, 128, 128), i32),
            pltpu.VMEM((5, 128, 128), i32),
            pltpu.SMEM((1,), i32),
            pltpu.VMEM((TQ // 2, D), i32),
            pltpu.VMEM((TQ // 2, D), i32),
            pltpu.VMEM((TQ // 2, D), i32),
            pltpu.VMEM((TQ // 2, D), i32),
            pltpu.VMEM((TQ // 2, F), i32),
            pltpu.VMEM((TQ // 2, F), i32),
            pltpu.VMEM((NG, TQ // 2, 128), i32),
            pltpu.VMEM((TQ // 4, 256, 128), f32),
            pltpu.VMEM((NB, D, 128), f32),
            pltpu.VMEM((TQ, D), f32),
            pltpu.VMEM((TQ // 2, D), i32),
            pltpu.VMEM((NG, TQ // 2, 128), i32),
            pltpu.VMEM((TQ, D), f32),
            pltpu.VMEM((TQ // 2, D), i32),
            pltpu.VMEM((F,), bf16),
            pltpu.VMEM((D,), bf16),
            pltpu.SemaphoreType.DMA((9,)),
            pltpu.SemaphoreType.DMA((NU,)),
            pltpu.SemaphoreType.DMA((NU + 2,)),
        ],
        compiler_params=pltpu.CompilerParams(
            dimension_semantics=("arbitrary",),
            vmem_limit_bytes=100 * 2**20),
    )(A_x, A_wqkv, A_wo, B_w1, B_b1, B_w2, B_b2)
```

```python
import functools
import math

import jax
import jax.numpy as jnp
from jax import lax
import jax.experimental.pallas as pl
import jax.experimental.pallas.tpu as pltpu

S = 2048
D = 640
F = 1536
H = 32
DH = 20
W = 256
NG = 8
TQ = 256
NB = TQ // 128
NU = S // TQ
EPS = 1e-5
QSCALE = (DH ** -0.5) * math.log2(math.e)
NEG_WORD = -243207808
ONE_WORD = 0x3F803F80
KS = 2
SS = 16
SD = 2

f32 = jnp.float32
bf16 = jnp.bfloat16
i32 = jnp.int32

CFG_FIRST = dict(
    DEPTH=2, REL=((0, 0), (0, 96), (0, 168)), WOD=3, VCH=4, MINT=4, ORDER='v,q',
    POS=(22, 24, 37, 41, 47, 47, 49, 49, 50),
    RELN={4: ((0, 0), (0, 120), (0, 168)), 9: ((0, 0), (0, 96), (0, 96)),
          10: ((0, 24), (0, 96), (0, 168)), 12: ((0, 0), (0, 96), (2, 24))})
CFG_MID = dict(
    DEPTH=2, REL=((0, 48), (0, 144), (0, 200)), WOD=4, VCH=8, MINT=4, ORDER='f1,f2a,f2b,k,v,q',
    POS=(4, 6, 7, 9, 10, 12, 13, 15, 18, 20, 21, 23, 24, 24, 27, 28, 30, 33, 33, 36, 37, 39,
         41, 41, 42, 42, 42, 42, 43, 43, 45, 45, 45, 45, 49, 49, 50, 50, 50, 50),
    RELN={3: ((0, 24), (0, 144), (0, 200)), 6: ((1, 144), (0, 144), (0, 200))})
CFG_LAST = dict(
    DEPTH=1, REL=((0, 24), (0, 120), (0, 240)), WOD=3, VCH=8, MINT=2, ORDER='f1,f2a,f2b',
    POS=(4, 7, 10, 13, 16, 19, 19, 22, 25, 27, 31, 31, 34, 38, 38, 38, 41, 44, 47, 47, 49, 50),
    RELN={5: ((0, 24), (0, 120), (0, 144)), 6: ((0, 24), (0, 96), (0, 24)),
          7: ((0, 24), (0, 96), (0, 240)), 9: ((0, 24), (1, 120), (0, 240)),
          10: ((0, 24), (3, 24), (0, 240))})
DMA_PLAN = dict(start='x0 x1 ka kb', x0='q', ka='v o', kb='w1 w2 x2 b1 b2 x3 x4 x5 x6 x7')


def _ln(x):
    m = jnp.mean(x, axis=-1, keepdims=True)
    xc = x - m
    v = jnp.mean(xc * xc, axis=-1, keepdims=True)
    return xc * lax.rsqrt(v + EPS)


def _gelu(x):
    c = math.sqrt(2.0 / math.pi)
    return 0.5 * x * (1.0 + jnp.tanh(c * (x + 0.044715 * (x * x * x))))


def _pack_pairs(a, odd, round_up):
    u = pltpu.bitcast(a, i32)
    if round_up:
        u = u + 0x8000
    rows = []
    for r in range(0, a.shape[0], 16):
        cols = []
        for c in range(0, a.shape[1], 128):
            lo = lax.shift_right_logical(u[r:r + 8, c:c + 128], 16)
            w = jnp.where(odd, pltpu.bitcast(u[r + 8:r + 16, c:c + 128], bf16),
                          pltpu.bitcast(lo, bf16))
            cols.append(pltpu.bitcast(w, i32))
        rows.append(cols[0] if len(cols) == 1 else jnp.concatenate(cols, axis=1))
    return rows[0] if len(rows) == 1 else jnp.concatenate(rows, axis=0)


def _odd_rows():
    return (lax.broadcasted_iota(i32, (16, 128), 0) & 1) == 1


def _words(a):
    return pltpu.bitcast(a.astype(bf16), i32)


def _as_bf16(w):
    return pltpu.bitcast(w, bf16)


def _group_tile(tiles, g, lane, zero_rest):
    lo = 80 * g
    t, off = lo // 128, lo % 128
    if off + 80 <= 128:
        if zero_rest:
            return jnp.where((lane >= off) & (lane < off + 80), tiles[t], 0)
        return tiles[t]
    e = off + 80 - 128
    if zero_rest:
        return jnp.where(lane < e, tiles[t + 1], jnp.where(lane >= off, tiles[t], 0))
    return jnp.where(lane < e, tiles[t + 1], tiles[t])


def _groups_ready(t):
    return [g for g in range(NG) if (80 * g + 79) // 128 == t]


def _sel(m, t, f_):
    if t is None and f_ is None:
        return None
    if t is None:
        t = 0
    if f_ is None:
        f_ = 0
    return jnp.where(m, t, f_)


class _Refs:
    pass


def _a_items(R, base, du, par, cfg, q_ref=None, free=False):
    st = {}
    xn_ref, xs_ref = R.xn[par], R.xs[par]
    q_ref = R.q if q_ref is None else q_ref
    row0 = base['krow'] + du * (TQ // 2)

    def ln1():
        x = R.x[pl.ds(base['xrow'] + du * TQ, TQ), :].astype(f32)
        xnf = _ln(x)
        xn_ref[...] = _words(xnf)
        xs_ref[...] = _pack_pairs(xnf, _odd_rows(), True)

    def kproj(t):
        k = jnp.dot(_as_bf16(xn_ref[...]), R.wk[:, 128 * t:128 * t + 128],
                    preferred_element_type=f32)
        st[('k', t)] = _words(k)
        lane = lax.broadcasted_iota(i32, (TQ // 2, 128), 1)
        tiles = {tt: st[('k', tt)] for tt in range(t + 1)}
        for g in _groups_ready(t):
            R.kg[g, pl.ds(row0 + W // 2, TQ // 2), :] = _group_tile(tiles, g, lane, True)

    def qproj(t):
        q = jnp.dot(_as_bf16(xn_ref[...]), R.wq[:, 128 * t:128 * t + 128],
                    preferred_element_type=f32) * QSCALE
        st[('q', t)] = _words(q)
        lane = lax.broadcasted_iota(i32, (TQ // 2, 128), 1)
        tiles = {tt: st[('q', tt)] for tt in range(t + 1)}
        for g in _groups_ready(t):
            q_ref[g] = _group_tile(tiles, g, lane, False)

    def vproj(c):
        gpc = NG // cfg['VCH']
        m0 = 80 * gpc * c
        vt = lax.dot_general(_as_bf16(R.wvt[m0 // 2:m0 // 2 + 40 * gpc, :]), _as_bf16(xs_ref[...]),
                             (((1,), (1,)), ((), ())), preferred_element_type=f32)
        vtw = _words(vt)
        sub8 = lax.broadcasted_iota(i32, (8, TQ), 0)
        pieces = []
        for gg in range(gpc):
            for hh in range(4):
                w0 = 40 * gg + 8 * hh
                a = vtw[w0:w0 + 8]
                b = vtw[w0 + 8:w0 + 16]
                if hh < 2:
                    b = jnp.where(sub8 >= 4, ONE_WORD, b)
                else:
                    a = jnp.where(sub8 < 4, ONE_WORD, a)
                pieces += [a, b]
        vtp = jnp.concatenate(pieces, axis=0)
        for nb in range(NB):
            R.vt[base['kb'] + du * NB + nb + 2, 64 * gpc * c:64 * gpc * (c + 1), :] = (
                vtp[:, 128 * nb:128 * nb + 128])

    return dict(
        ln=[('ln1', ln1, 0)],
        k=[('k', functools.partial(kproj, t), 320) for t in range(5)],
        q=[('q', functools.partial(qproj, t), 320,
            None if free else ('qk', NG + max(_groups_ready(t))), None) for t in range(5)],
        v=[('v', functools.partial(vproj, c), 1600 // cfg['VCH']) for c in range(cfg['VCH'])],
    )


def _b_items(R, base, du, cfg, z, q_ref=None, hbuf=0):
    st = {}
    s_ref, ot_ref = R.s, R.ot
    q_ref = R.q if q_ref is None else q_ref
    h1_ref, hn_ref = R.h1[hbuf], R.hn[hbuf]
    row0 = base['krow'] + du * (TQ // 2)
    DEPTH, MINT = cfg['DEPTH'], cfg['MINT']

    lane16 = lax.broadcasted_iota(i32, (16, 128), 1)
    r16 = lax.broadcasted_iota(i32, (16, 128), 0)
    cw = lane16 & 31
    odd16 = _odd_rows()
    tri0 = r16 > cw
    tri1 = r16 + 16 > cw
    rw = (r16 & 7) + 2 * (r16 & 8)
    m_old = (jnp.where(rw > cw, 0xFFFF, 0) | jnp.where(rw + 8 > cw, -65536, 0)).astype(i32)
    m_new = ~m_old
    s_odd = (lane16 & 32) != 0
    s_hi = (lane16 & 64) != 0
    sub8b = lax.broadcasted_iota(i32, (8, 128), 0) < 4

    def qk_stage(n):
        nb, g = n // NG, n % NG
        off = (80 * g) % 128
        rel = (lane16 - off) & 127
        cneg = jnp.where(rel == 80, NEG_WORD, 0).astype(i32)
        hmask = [(rel >= 20 * hh) & (rel < 20 * hh + 20) for hh in range(4)]
        for j in range(4):
            jj = 4 * nb + j
            qs = q_ref[g, 16 * jj:16 * jj + 16, :]
            bmat = _as_bf16(jnp.concatenate(
                [jnp.where(hmask[s ^ j], qs, cneg) for s in range(4)], axis=0))
            kw = R.kg[g, pl.ds(row0 + 16 * jj, 144), :]
            kwin = _as_bf16(jnp.concatenate(
                [kw[16:128], kw[0:8], kw[128:136], kw[8:16], kw[136:144]], axis=0))
            s_t = lax.dot_general(kwin, bmat, (((1,), (1,)), ((), ())),
                                  preferred_element_type=f32)
            slot = n * 4 + j
            e0 = jnp.where(tri0, s_t[224:240], s_t[240:256])
            e1 = jnp.where(tri1, s_t[256:272], s_t[272:288])
            sm = jnp.concatenate([s_t[0:224], e0, e1], axis=0)
            m = None
            for r in range(0, 256, 8):
                v = sm[r:r + 8]
                if m is None:
                    m = v
                    s_ref[slot, r:r + 8, :] = v
                else:
                    m = jnp.maximum(m, v)
                    tie = (r // 8) % MINT == MINT - 1
                    s_ref[slot, r:r + 8, :] = jnp.minimum(v, m) if tie else v
            st[('mx', n, j)] = jnp.max(m, axis=0, keepdims=True)
            st[('st', n, j)] = s_t

    def sm_stage(n):
        for j in range(4):
            slot = n * 4 + j
            mx = jnp.broadcast_to(st.pop(('mx', n, j)), (8, 128))
            hist = []
            for r in range(0, 256, SS):
                if len(hist) >= SD:
                    mx = jnp.maximum(mx, hist[-SD] - 3e38)
                p = jnp.exp2(s_ref[slot, r:r + SS, :] - jnp.concatenate([mx] * (SS // 8), axis=0))
                hist.append(p[SS - 8:SS])
                R.p[n % 3][j, r // 2:(r + SS) // 2, :] = _pack_pairs(p, odd16, False)

    def pv_stage(n):
        nb, g = n // NG, n % NG
        p_ref = R.p[n % 3]
        kb = base['kb'] + du * NB + nb
        acc = [None] * 4
        for t in range(3):
            spec = cfg['RELN'].get(n, cfg['REL'])[t]
            if spec is not None and ('st', n + DEPTH, spec[0]) in st:
                s_t = st[('st', n + DEPTH, spec[0])]
                p_ref[4, 8 * t:8 * t + 8, :] = pltpu.bitcast(s_t[spec[1]:spec[1] + 8], i32)

            def blk(j, b):
                if b < 0 or b > 8:
                    return None
                if b == 0:
                    return p_ref[z + j, 112:128, :] & m_old
                if b == 8:
                    return p_ref[z + j, 112:128, :] & m_new
                return p_ref[z + j, 16 * (b - 1):16 * b, :]

            wrows = [[], [], [], []]
            for a in range(4 * t, 4 * t + 4):
                X = [blk(j, a - j) for j in range(4)]
                Y = [_sel(s_odd, X[1], X[0]), _sel(s_odd, X[0], X[1]),
                     _sel(s_odd, X[3], X[2]), _sel(s_odd, X[2], X[3])]
                Z = [_sel(s_hi, Y[2], Y[0]), _sel(s_hi, Y[3], Y[1]),
                     _sel(s_hi, Y[0], Y[2]), _sel(s_hi, Y[1], Y[3])]
                for hh in range(4):
                    wrows[hh].append(Z[hh])
            for hh in range(4):
                h = 4 * g + hh
                wm = _as_bf16(jnp.concatenate(wrows[hh], axis=0))
                vl = _as_bf16(R.vt[kb + t, 16 * h:16 * h + 16, :])
                ot = jnp.dot(vl, wm, preferred_element_type=f32)
                acc[hh] = ot if acc[hh] is None else acc[hh] + ot
        on = []
        for hh in range(4):
            ot = acc[hh]
            den = ot[24:32] if hh < 2 else ot[0:8]
            r = 1.0 / den
            on.append([ot[8 * t:8 * t + 8] * r for t in range(4)])
        ot_ref[nb, 80 * g:80 * g + 80, :] = jnp.concatenate(
            [on[0][0], on[0][1], jnp.where(sub8b, on[0][2], on[1][0]),
             on[1][1], on[1][2], on[2][1], on[2][2],
             jnp.where(sub8b, on[2][3], on[3][1]), on[3][2], on[3][3]], axis=0)

    def wo_stage(nb):
        t = ot_ref[nb].T
        lane640 = lax.broadcasted_iota(i32, (32, D), 1)
        hid = lane640 // DH
        b0 = (hid & 1) != 0
        b1 = (hid & 2) != 0
        X = [t[32 * j:32 * j + 32] for j in range(4)]
        Y = [jnp.where(b0, X[j ^ 1], X[j]) for j in range(4)]
        Z = [jnp.where(b1, Y[j ^ 2], Y[j]) for j in range(4)]
        o = jnp.concatenate(Z, axis=0).astype(bf16)
        x = R.x[pl.ds(base['xrow'] + du * TQ + 128 * nb, 128), :].astype(f32)
        h1 = x + jnp.dot(o, R.wo[...], preferred_element_type=f32)
        h1_ref[128 * nb:128 * nb + 128, :] = h1
        hn_ref[64 * nb:64 * nb + 64, :] = _words(_ln(h1))

    items = []
    NA = NB * NG
    pend = []
    for n in range(NA + DEPTH):
        if n < NA:
            items.append(('qk', functools.partial(qk_stage, n), 288, n))
            items.append(('sm', functools.partial(sm_stage, n), 0))
        m = n - DEPTH
        if m >= 0:
            items.append(('pv', functools.partial(pv_stage, m), 96))
            if pend and n >= pend[0][0]:
                items.append(pend.pop(0)[1])
            if m % NG == NG - 1:
                pend.append((n + cfg['WOD'],
                             ('wo', functools.partial(wo_stage, m // NG), 800, m // NG)))
    items += [w[1] for w in pend]
    return items


def _c_items(R, base, du, par, hbuf=0, free=False):
    h1_ref, hn_ref, g_ref = R.h1[hbuf], R.hn[hbuf], R.g[par]
    w0, w1 = (None, None) if free else (('wo', 0), ('wo', 1))

    def f1(c):
        u = jnp.dot(_as_bf16(hn_ref[...]), R.w1[:, 128 * c:128 * c + 128],
                    preferred_element_type=f32)
        u = u + R.b1[128 * c:128 * c + 128].astype(f32).reshape(1, 128)
        g_ref[:, 128 * c:128 * c + 128] = _words(_gelu(u))

    def f2(m, n):
        g = _as_bf16(g_ref[64 * m:64 * m + 64, :])
        y = jnp.dot(g, R.w2[:, 128 * n:128 * n + 128], preferred_element_type=f32)
        y = y + R.b2[128 * n:128 * n + 128].astype(f32).reshape(1, 128)
        R.o[pl.ds(base['xrow'] + du * TQ + 128 * m, 128), 128 * n:128 * n + 128] = (
            h1_ref[128 * m:128 * m + 128, 128 * n:128 * n + 128] + y).astype(bf16)

    return dict(
        f1=[('f1', functools.partial(f1, c), 320, None, w0) for c in range(F // 128)],
        f2a=[('f2', functools.partial(f2, 0, n), 384, None, w0) for n in range(D // 128)],
        f2b=[('f2', functools.partial(f2, 1, n), 384, None, w1) for n in range(D // 128)],
    )


def _merge(main, fill, pos):
    assert len(pos) == len(fill) and list(pos) == sorted(pos)
    tags = {(it[0], it[3]): k for k, it in enumerate(main) if len(it) > 3}
    for p, it in zip(pos, fill):
        if len(it) == 5:
            assert it[3] is None or p > tags[it[3]]
            assert it[4] is None or p <= tags[it[4]]
    out = []
    for k in range(len(main) + 1):
        out += [it for p, it in zip(pos, fill) if p == k]
        if k < len(main):
            out.append(main[k])
    return out


def _phase(parts, main, cfg):
    fill = []
    for key in cfg['ORDER'].split(','):
        fill += parts.get(key, [])
    pre = parts.get('ln', [])
    if main is None:
        return pre + fill
    return pre + _merge(main, fill, cfg['POS'])


def _run(items):
    for it in items:
        it[1]()


def _kernel(x_hbm, wqkv_hbm, wo_hbm, w1_hbm, b1_hbm, w2_hbm, b2_hbm, o_hbm,
            x_ref, o_ref, kg_ref, vt_ref, wvt_ref, wq_ref, wk_ref, wv_ref, wo_ref, w1_ref, w2_ref,
            p0_ref, p1_ref, p2_ref, z_ref,
            xn0, xn1, xs0, xs1, g0, g1, q_ref, s_ref, ot_ref, h1_ref, hn_ref,
            qa_ref, h1a_ref, hna_ref, b1_ref, b2_ref,
            sem, xsem, osem):
    i = pl.program_id(0)
    R = _Refs()
    R.x, R.o, R.kg, R.vt, R.wvt = x_ref, o_ref, kg_ref, vt_ref, wvt_ref
    R.wq, R.wk, R.wo, R.w1, R.w2, R.b1, R.b2 = wq_ref, wk_ref, wo_ref, w1_ref, w2_ref, b1_ref, b2_ref
    R.p = (p0_ref, p1_ref, p2_ref)
    R.xn, R.xs, R.g = (xn0, xn1), (xs0, xs1), (g0, g1)
    R.q, R.s, R.ot = q_ref, s_ref, ot_ref
    R.h1, R.hn = (h1_ref, h1a_ref), (hn_ref, hna_ref)

    def xcopy(b):
        return pltpu.make_async_copy(x_hbm.at[0, pl.ds(b * TQ, TQ), :],
                                     x_ref.at[pl.ds(b * TQ, TQ), :], xsem.at[b])

    def ocopy(b):
        return pltpu.make_async_copy(o_ref.at[pl.ds(b * TQ, TQ), :],
                                     o_hbm.at[0, pl.ds(b * TQ, TQ), :], osem.at[b])

    def static_base(u):
        return dict(krow=u * (TQ // 2), xrow=u * TQ, kb=u * NB)

    def opaque_zero():
        return jnp.clip(z_ref[0], 0, 1)

    @pl.when(i == 0)
    def _first():
        cfg = CFG_FIRST
        specs = dict(
            ka=(wqkv_hbm, D, wk_ref, 0, 128 * KS), kb=(wqkv_hbm, D, wk_ref, 128 * KS, D - 128 * KS),
            q=(wqkv_hbm, 0, wq_ref, 0, D), v=(wqkv_hbm, 2 * D, wv_ref, 0, D),
            o=(wo_hbm, 0, wo_ref, 0, D), w1=(w1_hbm, 0, w1_ref, 0, F), w2=(w2_hbm, 0, w2_ref, 0, D))
        copies = {}
        for n, (name, (src, c0, dst, d0, nc)) in enumerate(specs.items()):
            copies[name] = pltpu.make_async_copy(
                src.at[:, pl.ds(c0 + d0, nc)], dst.at[:, pl.ds(d0, nc)], sem.at[n])
        copies['b1'] = pltpu.make_async_copy(b1_hbm, b1_ref, sem.at[7])
        copies['b2'] = pltpu.make_async_copy(b2_hbm, b2_ref, sem.at[8])

        def go(p):
            for name in DMA_PLAN.get(p, '').split():
                if name[0] == 'x':
                    xcopy(int(name[1:])).start()
                else:
                    copies[name].start()

        def wait(name):
            copies[name].wait()
            go(name)

        go('start')
        z_ref[0] = 0
        lane1 = lax.broadcasted_iota(i32, (W // 2, 128), 1)
        for g in range(NG):
            sp = (80 * g + 80) % 128
            kg_ref[g, 0:W // 2, :] = jnp.where(lane1 == sp, ONE_WORD, 0).astype(i32)
        vt_ref[0:2] = jnp.zeros((2, H * 16, 128), i32)
        for p_ref in R.p:
            p_ref[...] = jnp.zeros(p_ref.shape, i32)
        xcopy(0).wait()
        go('x0')
        base = static_base(0)
        a0 = _a_items(R, base, 0, 0, cfg, q_ref=qa_ref)
        a1 = _a_items(R, base, 1, 1, cfg, free=True)
        _run(a0['ln'])
        xcopy(1).wait()
        wait('ka')
        _run(a0['k'][:KS] + a1['ln'] + a1['k'][:KS])
        wait('kb')
        _run(a0['k'][KS:] + a1['k'][KS:])
        wait('q')
        _run(a0['q'])
        items = _phase(dict(q=a1['q'], v=a1['v']),
                       _b_items(R, base, 0, cfg, opaque_zero(), q_ref=qa_ref), cfg)
        lead = [it for it in items if it[0] in ('qk', 'sm')][:4]
        items = [it for it in items if not any(it is l for l in lead)]
        k = next(n for n, it in enumerate(items) if it[0] == 'pv')
        _run(lead)
        wait('v')
        wait('o')
        wvt_ref[...] = _words(wv_ref[...].astype(f32).T)
        _run(items[:k] + a0['v'] + items[k:])
        wait('w1')
        wait('w2')
        wait('b1')
        wait('b2')

    @pl.when((i > 0) & (i < NU - 1))
    def _mid():
        cfg = CFG_MID
        xcopy(i + 1).wait()
        base = dict(krow=pl.multiple_of((i - 1) * (TQ // 2), TQ // 2),
                    xrow=pl.multiple_of((i - 1) * TQ, TQ), kb=(i - 1) * NB)
        z = opaque_zero()
        parts = _a_items(R, base, 2, 0, cfg)
        parts.update(_c_items(R, base, 0, 0))
        _run(_phase(parts, _b_items(R, base, 1, cfg, z), cfg))
        ocopy(i - 1).start()

    @pl.when(i == NU - 1)
    def _last():
        cfg = CFG_LAST
        base = static_base(NU - 2)
        z = opaque_zero()
        _run(_phase(_c_items(R, base, 0, 0, free=True), _b_items(R, base, 1, cfg, z, hbuf=1), cfg))
        ocopy(NU - 2).start()
        r0 = (NU - 1) * TQ
        pieces = {16: (r0, 0, D), 20: (r0 + 128, 0, 512), 21: (r0 + 128, 512, D - 512)}
        tail = []
        for n, it in enumerate(_phase(_c_items(R, base, 1, 1, hbuf=1), None, cfg)):
            it[1]()
            if n in pieces:
                r, c, nc = pieces[n]
                cp = pltpu.make_async_copy(o_ref.at[pl.ds(r, 128), pl.ds(c, nc)],
                                           o_hbm.at[0, pl.ds(r, 128), pl.ds(c, nc)],
                                           osem.at[NU - 1 + len(tail)])
                cp.start()
                tail.append(cp)
        for b in range(NU - 1):
            ocopy(b).wait()
        for cp in tail:
            cp.wait()


@jax.jit
def pallas_sequential_preLN__sliding_block__dense_activation_gelu__prompt_kernel(
    A_x: jax.Array,
    A_wqkv: jax.Array,
    A_wo: jax.Array,
    B_x: jax.Array,
    B_w1: jax.Array,
    B_b1: jax.Array,
    B_w2: jax.Array,
    B_b2: jax.Array,
):
    del B_x
    hbm = pl.BlockSpec(memory_space=pl.ANY)
    return pl.pallas_call(
        _kernel,
        grid=(NU,),
        in_specs=[hbm] * 7,
        out_specs=hbm,
        out_shape=jax.ShapeDtypeStruct((1, S, D), bf16),
        scratch_shapes=[
            pltpu.VMEM((S, D), bf16),
            pltpu.VMEM((S, D), bf16),
            pltpu.VMEM((NG, (S + W) // 2, 128), i32),
            pltpu.VMEM((S // 128 + 2, H * 16, 128), i32),
            pltpu.VMEM((D // 2, D), i32),
            pltpu.VMEM((D, D), bf16),
            pltpu.VMEM((D, D), bf16),
            pltpu.VMEM((D, D), bf16),
            pltpu.VMEM((D, D), bf16),
            pltpu.VMEM((D, F), bf16),
            pltpu.VMEM((F, D), bf16),
            pltpu.VMEM((5, 128, 128), i32),
            pltpu.VMEM((5, 128, 128), i32),
            pltpu.VMEM((5, 128, 128), i32),
            pltpu.SMEM((1,), i32),
            pltpu.VMEM((TQ // 2, D), i32),
            pltpu.VMEM((TQ // 2, D), i32),
            pltpu.VMEM((TQ // 2, D), i32),
            pltpu.VMEM((TQ // 2, D), i32),
            pltpu.VMEM((TQ // 2, F), i32),
            pltpu.VMEM((TQ // 2, F), i32),
            pltpu.VMEM((NG, TQ // 2, 128), i32),
            pltpu.VMEM((TQ // 4, 256, 128), f32),
            pltpu.VMEM((NB, D, 128), f32),
            pltpu.VMEM((TQ, D), f32),
            pltpu.VMEM((TQ // 2, D), i32),
            pltpu.VMEM((NG, TQ // 2, 128), i32),
            pltpu.VMEM((TQ, D), f32),
            pltpu.VMEM((TQ // 2, D), i32),
            pltpu.VMEM((F,), bf16),
            pltpu.VMEM((D,), bf16),
            pltpu.SemaphoreType.DMA((9,)),
            pltpu.SemaphoreType.DMA((NU,)),
            pltpu.SemaphoreType.DMA((NU + 2,)),
        ],
        compiler_params=pltpu.CompilerParams(
            dimension_semantics=("arbitrary",),
            vmem_limit_bytes=100 * 2**20,
            disable_semaphore_checks=True),
    )(A_x, A_wqkv, A_wo, B_w1, B_b1, B_w2, B_b2)
```

```python
import functools
import math

import jax
import jax.numpy as jnp
from jax import lax
import jax.experimental.pallas as pl
import jax.experimental.pallas.tpu as pltpu

S = 2048
D = 640
F = 1536
H = 32
DH = 20
W = 256
NG = 8
TQ = 256
NB = TQ // 128
NU = S // TQ
EPS = 1e-5
QSCALE = (DH ** -0.5) * math.log2(math.e)
ONE_WORD = 0x3F803F80
KS = 2

f32 = jnp.float32
bf16 = jnp.bfloat16
i32 = jnp.int32

CFG_FIRST = dict(
    DEPTH=2, REL=((0, 48), None, None), WOD=2, VCH=4, MINT=4, SS=32, SD=3, ORDER='v,q',
    POS=(14, 25, 30, 37, 45, 49, 50, 50, 50),
    RELN={0: ((2, 120), None, None), 4: ((2, 24), None, None)})
CFG_MID = dict(
    DEPTH=2, REL=((0, 48), (0, 144), (0, 200)), WOD=4, VCH=8, MINT=4, SS=16, SD=2,
    ORDER='f1,f2a,f2b,k,v,q',
    POS=(4, 6, 7, 9, 10, 12, 13, 15, 18, 20, 21, 23, 24, 24, 27, 28, 30, 33, 33, 36, 39, 41,
         41, 41, 42, 42, 42, 42, 43, 45, 45, 45, 45, 45, 49, 49, 50, 50, 50, 50),
    RELN={3: ((0, 24), (0, 144), (0, 200)), 6: ((1, 144), (0, 144), (0, 200)),
          8: ((0, 48), (0, 144), (2, 96))})
CFG_LAST = dict(
    DEPTH=1, REL=((0, 24), (0, 120), (0, 240)), WOD=3, VCH=8, MINT=2, SS=16, SD=2,
    ORDER='f1,f2a,f2b',
    POS=(4, 7, 10, 13, 16, 19, 19, 22, 25, 27, 31, 31, 34, 38, 38, 38, 41, 44, 47, 47, 49, 50),
    RELN={0: ((0, 24), None, (0, 240)), 5: ((0, 24), (0, 120), (0, 144)),
          6: ((0, 24), (0, 96), (0, 216)), 7: ((0, 24), (0, 96), (0, 240)),
          9: ((0, 24), (1, 120), (0, 240)), 10: ((0, 24), (0, 72), (0, 240)),
          11: ((1, 48), (0, 72), (0, 240))})
DMA_PLAN = dict(start='x0 x1 ka kb', x0='q', ka='v o', kb='w1 w2 x2 b1 b2',
                end='x3 x4 x5 x6 x7')


def _ln(x):
    m = jnp.mean(x, axis=-1, keepdims=True)
    xc = x - m
    v = jnp.mean(xc * xc, axis=-1, keepdims=True)
    return xc * lax.rsqrt(v + EPS)


def _gelu(x):
    c = math.sqrt(2.0 / math.pi)
    return 0.5 * x * (1.0 + jnp.tanh(c * (x + 0.044715 * (x * x * x))))


def _pack_pairs(a, odd, round_up):
    u = pltpu.bitcast(a, i32)
    if round_up:
        u = u + 0x8000
    rows = []
    for r in range(0, a.shape[0], 16):
        cols = []
        for c in range(0, a.shape[1], 128):
            lo = lax.shift_right_logical(u[r:r + 8, c:c + 128], 16)
            w = jnp.where(odd, pltpu.bitcast(u[r + 8:r + 16, c:c + 128], bf16),
                          pltpu.bitcast(lo, bf16))
            cols.append(pltpu.bitcast(w, i32))
        rows.append(cols[0] if len(cols) == 1 else jnp.concatenate(cols, axis=1))
    return rows[0] if len(rows) == 1 else jnp.concatenate(rows, axis=0)


def _odd_rows():
    return (lax.broadcasted_iota(i32, (16, 128), 0) & 1) == 1


def _words(a):
    return pltpu.bitcast(a.astype(bf16), i32)


def _as_bf16(w):
    return pltpu.bitcast(w, bf16)


def _group_tile(tiles, g, lane):
    lo = 80 * g
    t, off = lo // 128, lo % 128
    if off + 80 <= 128:
        return tiles[t]
    return jnp.where(lane < off + 80 - 128, tiles[t + 1], tiles[t])


def _groups_ready(t):
    return [g for g in range(NG) if (80 * g + 79) // 128 == t]


def _sel(m, t, f_):
    if t is None and f_ is None:
        return None
    if t is None:
        t = 0
    if f_ is None:
        f_ = 0
    return jnp.where(m, t, f_)


class _Refs:
    pass


def _a_items(R, base, du, par, cfg, q_ref=None, free=False):
    st = {}
    xn_ref, xs_ref = R.xn[par], R.xs[par]
    q_ref = R.q if q_ref is None else q_ref
    row0 = base['krow'] + du * (TQ // 2)

    def ln1():
        x = R.x[pl.ds(base['xrow'] + du * TQ, TQ), :].astype(f32)
        xnf = _ln(x)
        xn_ref[...] = _words(xnf)
        xs_ref[...] = _pack_pairs(xnf, _odd_rows(), True)

    def kproj(t):
        k = jnp.dot(_as_bf16(xn_ref[...]), R.wk[:, 128 * t:128 * t + 128],
                    preferred_element_type=f32)
        st[('k', t)] = _words(k)
        lane = lax.broadcasted_iota(i32, (TQ // 2, 128), 1)
        tiles = {tt: st[('k', tt)] for tt in range(t + 1)}
        for g in _groups_ready(t):
            R.kg[g, pl.ds(row0 + W // 2, TQ // 2), :] = _group_tile(tiles, g, lane)

    def qproj(t):
        q = jnp.dot(_as_bf16(xn_ref[...]), R.wq[:, 128 * t:128 * t + 128],
                    preferred_element_type=f32) * QSCALE
        st[('q', t)] = _words(q)
        lane = lax.broadcasted_iota(i32, (TQ // 2, 128), 1)
        tiles = {tt: st[('q', tt)] for tt in range(t + 1)}
        for g in _groups_ready(t):
            q_ref[g] = _group_tile(tiles, g, lane)

    def vproj(c):
        gpc = NG // cfg['VCH']
        m0 = 80 * gpc * c
        vt = lax.dot_general(_as_bf16(R.wvt[m0 // 2:m0 // 2 + 40 * gpc, :]), _as_bf16(xs_ref[...]),
                             (((1,), (1,)), ((), ())), preferred_element_type=f32)
        vtw = _words(vt)
        sub8 = lax.broadcasted_iota(i32, (8, TQ), 0)
        pieces = []
        for gg in range(gpc):
            for hh in range(4):
                w0 = 40 * gg + 8 * hh
                a = vtw[w0:w0 + 8]
                b = vtw[w0 + 8:w0 + 16]
                if hh < 2:
                    b = jnp.where(sub8 >= 4, ONE_WORD, b)
                else:
                    a = jnp.where(sub8 < 4, ONE_WORD, a)
                pieces += [a, b]
        vtp = jnp.concatenate(pieces, axis=0)
        for nb in range(NB):
            R.vt[base['kb'] + du * NB + nb + 2, 64 * gpc * c:64 * gpc * (c + 1), :] = (
                vtp[:, 128 * nb:128 * nb + 128])

    return dict(
        ln=[('ln1', ln1, 0)],
        k=[('k', functools.partial(kproj, t), 320) for t in range(5)],
        q=[('q', functools.partial(qproj, t), 320,
            None if free else ('qk', NG + max(_groups_ready(t))), None) for t in range(5)],
        v=[('v', functools.partial(vproj, c), 1600 // cfg['VCH']) for c in range(cfg['VCH'])],
    )


def _b_items(R, base, du, cfg, z, q_ref=None, hbuf=0, head=False):
    st = {}
    s_ref, ot_ref = R.s, R.ot
    q_ref = R.q if q_ref is None else q_ref
    h1_ref, hn_ref = R.h1[hbuf], R.hn[hbuf]
    row0 = base['krow'] + du * (TQ // 2)
    DEPTH, MINT, SS, SD = cfg['DEPTH'], cfg['MINT'], cfg['SS'], cfg['SD']

    lane16 = lax.broadcasted_iota(i32, (16, 128), 1)
    r16 = lax.broadcasted_iota(i32, (16, 128), 0)
    cw = lane16 & 31
    odd16 = _odd_rows()
    tri0 = r16 > cw
    tri1 = r16 + 16 > cw
    rw = (r16 & 7) + 2 * (r16 & 8)
    m_old = (jnp.where(rw > cw, 0xFFFF, 0) | jnp.where(rw + 8 > cw, -65536, 0)).astype(i32)
    m_new = ~m_old
    s_odd = (lane16 & 32) != 0
    s_hi = (lane16 & 64) != 0
    sub8b = lax.broadcasted_iota(i32, (8, 128), 0) < 4

    def qk_stage(n):
        nb, g = n // NG, n % NG
        off = (80 * g) % 128
        rel = (lane16 - off) & 127
        hmask = [(rel >= 20 * hh) & (rel < 20 * hh + 20) for hh in range(4)]
        for j in range(4):
            jj = 4 * nb + j
            qs = q_ref[g, 16 * jj:16 * jj + 16, :]
            bmat = _as_bf16(jnp.concatenate(
                [jnp.where(hmask[s ^ j], qs, 0) for s in range(4)], axis=0))
            slot = n * 4 + j
            if head:
                kwin = _as_bf16(R.kg[g, W // 2:W // 2 + 16 * jj + 16, :])
                s_t = lax.dot_general(kwin, bmat, (((1,), (1,)), ((), ())),
                                      preferred_element_type=f32)
                e0 = jnp.where(tri0, -1e30, s_t[32 * jj:32 * jj + 16])
                e1 = jnp.where(tri1, -1e30, s_t[32 * jj + 16:32 * jj + 32])
                sm = jnp.concatenate(([s_t[0:32 * jj]] if jj else []) + [e0, e1], axis=0)
                r0 = 224 - 32 * jj
            else:
                kw = R.kg[g, pl.ds(row0 + 16 * jj, 144), :]
                kwin = _as_bf16(jnp.concatenate(
                    [kw[16:128], kw[0:8], kw[128:136], kw[8:16], kw[136:144]], axis=0))
                s_t = lax.dot_general(kwin, bmat, (((1,), (1,)), ((), ())),
                                      preferred_element_type=f32)
                e0 = jnp.where(tri0, s_t[224:240], s_t[240:256])
                e1 = jnp.where(tri1, s_t[256:272], s_t[272:288])
                sm = jnp.concatenate([s_t[0:224], e0, e1], axis=0)
                r0 = 0
            m = None
            for r in range(r0, 256, 8):
                v = sm[r - r0:r - r0 + 8]
                if m is None:
                    m = v
                    s_ref[slot, r:r + 8, :] = v
                else:
                    m = jnp.maximum(m, v)
                    tie = (r // 8) % MINT == MINT - 1
                    s_ref[slot, r:r + 8, :] = jnp.minimum(v, m) if tie else v
            st[('mx', n, j)] = jnp.max(m, axis=0, keepdims=True)
            st[('st', n, j)] = s_t

    def sm_stage(n):
        for j in range(4):
            slot = n * 4 + j
            mx = jnp.broadcast_to(st.pop(('mx', n, j)), (8, 128))
            hist = []
            r0 = 224 - 32 * (4 * (n // NG) + j) if head else 0
            for r in range(r0, 256, SS):
                if len(hist) >= SD:
                    mx = jnp.maximum(mx, hist[-SD] - 3e38)
                p = jnp.exp2(s_ref[slot, r:r + SS, :] - jnp.concatenate([mx] * (SS // 8), axis=0))
                hist.append(p[SS - 8:SS])
                R.p[n % 3][j, r // 2:(r + SS) // 2, :] = _pack_pairs(p, odd16, False)

    def pv_stage(n):
        nb, g = n // NG, n % NG
        p_ref = R.p[n % 3]
        kb = base['kb'] + du * NB + nb
        acc = [None] * 4
        for t in range(2 - nb if head else 0, 3):
            spec = cfg['RELN'].get(n, cfg['REL'])[t]
            if spec is not None and ('st', n + DEPTH, spec[0]) in st:
                s_t = st[('st', n + DEPTH, spec[0])]
                rr = min(spec[1], s_t.shape[0] - 8)
                p_ref[4, 8 * t:8 * t + 8, :] = pltpu.bitcast(s_t[rr:rr + 8], i32)

            def blk(j, b):
                if b < 0 or b > 8 or (head and b < 8 - 4 * nb - j):
                    return None
                if b == 0:
                    return p_ref[z + j, 112:128, :] & m_old
                if b == 8:
                    return p_ref[z + j, 112:128, :] & m_new
                return p_ref[z + j, 16 * (b - 1):16 * b, :]

            wrows = [[], [], [], []]
            for a in range(4 * t, 4 * t + 4):
                X = [blk(j, a - j) for j in range(4)]
                Y = [_sel(s_odd, X[1], X[0]), _sel(s_odd, X[0], X[1]),
                     _sel(s_odd, X[3], X[2]), _sel(s_odd, X[2], X[3])]
                Z = [_sel(s_hi, Y[2], Y[0]), _sel(s_hi, Y[3], Y[1]),
                     _sel(s_hi, Y[0], Y[2]), _sel(s_hi, Y[1], Y[3])]
                for hh in range(4):
                    wrows[hh].append(Z[hh])
            for hh in range(4):
                h = 4 * g + hh
                wm = _as_bf16(jnp.concatenate(wrows[hh], axis=0))
                vl = _as_bf16(R.vt[kb + t, 16 * h:16 * h + 16, :])
                ot = jnp.dot(vl, wm, preferred_element_type=f32)
                acc[hh] = ot if acc[hh] is None else acc[hh] + ot
        on = []
        for hh in range(4):
            ot = acc[hh]
            den = ot[24:32] if hh < 2 else ot[0:8]
            r = 1.0 / den
            on.append([ot[8 * t:8 * t + 8] * r for t in range(4)])
        ot_ref[nb, 80 * g:80 * g + 80, :] = jnp.concatenate(
            [on[0][0], on[0][1], jnp.where(sub8b, on[0][2], on[1][0]),
             on[1][1], on[1][2], on[2][1], on[2][2],
             jnp.where(sub8b, on[2][3], on[3][1]), on[3][2], on[3][3]], axis=0)

    def wo_stage(nb):
        t = ot_ref[nb].T
        lane640 = lax.broadcasted_iota(i32, (32, D), 1)
        hid = lane640 // DH
        b0 = (hid & 1) != 0
        b1 = (hid & 2) != 0
        X = [t[32 * j:32 * j + 32] for j in range(4)]
        Y = [jnp.where(b0, X[j ^ 1], X[j]) for j in range(4)]
        Z = [jnp.where(b1, Y[j ^ 2], Y[j]) for j in range(4)]
        o = jnp.concatenate(Z, axis=0).astype(bf16)
        x = R.x[pl.ds(base['xrow'] + du * TQ + 128 * nb, 128), :].astype(f32)
        h1 = x + jnp.dot(o, R.wo[...], preferred_element_type=f32)
        h1_ref[128 * nb:128 * nb + 128, :] = h1
        hn_ref[64 * nb:64 * nb + 64, :] = _words(_ln(h1))

    items = []
    NA = NB * NG
    pend = []
    for n in range(NA + DEPTH):
        if n < NA:
            items.append(('qk', functools.partial(qk_stage, n), 288, n))
            items.append(('sm', functools.partial(sm_stage, n), 0))
        m = n - DEPTH
        if m >= 0:
            items.append(('pv', functools.partial(pv_stage, m), 96))
            if pend and n >= pend[0][0]:
                items.append(pend.pop(0)[1])
            if m % NG == NG - 1:
                pend.append((n + cfg['WOD'],
                             ('wo', functools.partial(wo_stage, m // NG), 800, m // NG)))
    items += [w[1] for w in pend]
    return items


def _c_items(R, base, du, par, hbuf=0, free=False):
    h1_ref, hn_ref, g_ref = R.h1[hbuf], R.hn[hbuf], R.g[par]
    w0, w1 = (None, None) if free else (('wo', 0), ('wo', 1))

    def f1(c):
        u = jnp.dot(_as_bf16(hn_ref[...]), R.w1[:, 128 * c:128 * c + 128],
                    preferred_element_type=f32)
        u = u + R.b1[128 * c:128 * c + 128].astype(f32).reshape(1, 128)
        g_ref[:, 128 * c:128 * c + 128] = _words(_gelu(u))

    def f2(m, n):
        g = _as_bf16(g_ref[64 * m:64 * m + 64, :])
        y = jnp.dot(g, R.w2[:, 128 * n:128 * n + 128], preferred_element_type=f32)
        y = y + R.b2[128 * n:128 * n + 128].astype(f32).reshape(1, 128)
        R.o[pl.ds(base['xrow'] + du * TQ + 128 * m, 128), 128 * n:128 * n + 128] = (
            h1_ref[128 * m:128 * m + 128, 128 * n:128 * n + 128] + y).astype(bf16)

    return dict(
        f1=[('f1', functools.partial(f1, c), 320, None, w0) for c in range(F // 128)],
        f2a=[('f2', functools.partial(f2, 0, n), 384, None, w0) for n in range(D // 128)],
        f2b=[('f2', functools.partial(f2, 1, n), 384, None, w1) for n in range(D // 128)],
    )


def _merge(main, fill, pos):
    assert len(pos) == len(fill) and list(pos) == sorted(pos)
    tags = {(it[0], it[3]): k for k, it in enumerate(main) if len(it) > 3}
    for p, it in zip(pos, fill):
        if len(it) == 5:
            assert it[3] is None or p > tags[it[3]]
            assert it[4] is None or p <= tags[it[4]]
    out = []
    for k in range(len(main) + 1):
        out += [it for p, it in zip(pos, fill) if p == k]
        if k < len(main):
            out.append(main[k])
    return out


def _phase(parts, main, cfg):
    fill = []
    for key in cfg['ORDER'].split(','):
        fill += parts.get(key, [])
    pre = parts.get('ln', [])
    if main is None:
        return pre + fill
    return pre + _merge(main, fill, cfg['POS'])


def _run(items):
    for it in items:
        it[1]()


def _kernel(x_hbm, wqkv_hbm, wo_hbm, w1_hbm, b1_hbm, w2_hbm, b2_hbm, o_hbm,
            x_ref, o_ref, kg_ref, vt_ref, wvt_ref, wq_ref, wk_ref, wv_ref, wo_ref, w1_ref, w2_ref,
            p0_ref, p1_ref, p2_ref, z_ref,
            xn0, xn1, xs0, xs1, g0, g1, q_ref, s_ref, ot_ref, h1_ref, hn_ref,
            qa_ref, h1a_ref, hna_ref, b1_ref, b2_ref,
            sem, xsem, osem):
    i = pl.program_id(0)
    R = _Refs()
    R.x, R.o, R.kg, R.vt, R.wvt = x_ref, o_ref, kg_ref, vt_ref, wvt_ref
    R.wq, R.wk, R.wo, R.w1, R.w2, R.b1, R.b2 = wq_ref, wk_ref, wo_ref, w1_ref, w2_ref, b1_ref, b2_ref
    R.p = (p0_ref, p1_ref, p2_ref)
    R.xn, R.xs, R.g = (xn0, xn1), (xs0, xs1), (g0, g1)
    R.q, R.s, R.ot = q_ref, s_ref, ot_ref
    R.h1, R.hn = (h1_ref, h1a_ref), (hn_ref, hna_ref)

    def xcopy(b):
        return pltpu.make_async_copy(x_hbm.at[0, pl.ds(b * TQ, TQ), :],
                                     x_ref.at[pl.ds(b * TQ, TQ), :], xsem.at[b])

    def ocopy(b):
        return pltpu.make_async_copy(o_ref.at[pl.ds(b * TQ, TQ), :],
                                     o_hbm.at[0, pl.ds(b * TQ, TQ), :], osem.at[b])

    def static_base(u):
        return dict(krow=u * (TQ // 2), xrow=u * TQ, kb=u * NB)

    def opaque_zero():
        return jnp.clip(z_ref[0], 0, 1)

    @pl.when(i == 0)
    def _first():
        cfg = CFG_FIRST
        specs = dict(
            ka=(wqkv_hbm, D, wk_ref, 0, 128 * KS), kb=(wqkv_hbm, D, wk_ref, 128 * KS, D - 128 * KS),
            q=(wqkv_hbm, 0, wq_ref, 0, D), v=(wqkv_hbm, 2 * D, wv_ref, 0, D),
            o=(wo_hbm, 0, wo_ref, 0, D), w1=(w1_hbm, 0, w1_ref, 0, F), w2=(w2_hbm, 0, w2_ref, 0, D))
        copies = {}
        for n, (name, (src, c0, dst, d0, nc)) in enumerate(specs.items()):
            copies[name] = pltpu.make_async_copy(
                src.at[:, pl.ds(c0 + d0, nc)], dst.at[:, pl.ds(d0, nc)], sem.at[n])
        copies['b1'] = pltpu.make_async_copy(b1_hbm, b1_ref, sem.at[7])
        copies['b2'] = pltpu.make_async_copy(b2_hbm, b2_ref, sem.at[8])

        def go(p):
            for name in DMA_PLAN.get(p, '').split():
                if name[0] == 'x':
                    xcopy(int(name[1:])).start()
                else:
                    copies[name].start()

        def wait(name):
            copies[name].wait()
            go(name)

        go('start')
        z_ref[0] = 0
        for p_ref in R.p:
            p_ref[...] = jnp.zeros(p_ref.shape, i32)
        xcopy(0).wait()
        go('x0')
        base = static_base(0)
        a0 = _a_items(R, base, 0, 0, cfg, q_ref=qa_ref)
        a1 = _a_items(R, base, 1, 1, cfg, free=True)
        _run(a0['ln'])
        xcopy(1).wait()
        wait('ka')
        _run(a0['k'][:KS] + a1['ln'] + a1['k'][:KS])
        wait('kb')
        _run(a0['k'][KS:] + a1['k'][KS:])
        wait('q')
        _run(a0['q'])
        items = _phase(dict(q=a1['q'], v=a1['v']),
                       _b_items(R, base, 0, cfg, opaque_zero(), q_ref=qa_ref, head=True), cfg)
        lead = [it for it in items if it[0] in ('qk', 'sm')][:4]
        items = [it for it in items if not any(it is l for l in lead)]
        k = next(n for n, it in enumerate(items) if it[0] == 'pv')
        _run(lead)
        wait('v')
        wait('o')
        wvt_ref[...] = _words(wv_ref[...].astype(f32).T)
        _run(items[:k] + a0['v'] + items[k:])
        go('end')
        wait('w1')
        wait('w2')
        wait('b1')
        wait('b2')

    @pl.when((i > 0) & (i < NU - 1))
    def _mid():
        cfg = CFG_MID
        xcopy(i + 1).wait()
        base = dict(krow=pl.multiple_of((i - 1) * (TQ // 2), TQ // 2),
                    xrow=pl.multiple_of((i - 1) * TQ, TQ), kb=(i - 1) * NB)
        z = opaque_zero()
        parts = _a_items(R, base, 2, 0, cfg)
        parts.update(_c_items(R, base, 0, 0))
        _run(_phase(parts, _b_items(R, base, 1, cfg, z), cfg))
        ocopy(i - 1).start()

    @pl.when(i == NU - 1)
    def _last():
        cfg = CFG_LAST
        base = static_base(NU - 2)
        z = opaque_zero()
        _run(_phase(_c_items(R, base, 0, 0, free=True), _b_items(R, base, 1, cfg, z, hbuf=1), cfg))
        ocopy(NU - 2).start()
        r0 = (NU - 1) * TQ
        pieces = {16: (r0, 0, D), 20: (r0 + 128, 0, 512), 21: (r0 + 128, 512, D - 512)}
        tail = []
        for n, it in enumerate(_phase(_c_items(R, base, 1, 1, hbuf=1), None, cfg)):
            it[1]()
            if n in pieces:
                r, c, nc = pieces[n]
                cp = pltpu.make_async_copy(o_ref.at[pl.ds(r, 128), pl.ds(c, nc)],
                                           o_hbm.at[0, pl.ds(r, 128), pl.ds(c, nc)],
                                           osem.at[NU - 1 + len(tail)])
                cp.start()
                tail.append(cp)
        for b in range(NU - 1):
            ocopy(b).wait()
        for cp in tail:
            cp.wait()


@jax.jit
def pallas_sequential_preLN__sliding_block__dense_activation_gelu__prompt_kernel(
    A_x: jax.Array,
    A_wqkv: jax.Array,
    A_wo: jax.Array,
    B_x: jax.Array,
    B_w1: jax.Array,
    B_b1: jax.Array,
    B_w2: jax.Array,
    B_b2: jax.Array,
):
    del B_x
    hbm = pl.BlockSpec(memory_space=pl.ANY)
    return pl.pallas_call(
        _kernel,
        grid=(NU,),
        in_specs=[hbm] * 7,
        out_specs=hbm,
        out_shape=jax.ShapeDtypeStruct((1, S, D), bf16),
        scratch_shapes=[
            pltpu.VMEM((S, D), bf16),
            pltpu.VMEM((S, D), bf16),
            pltpu.VMEM((NG, (S + W) // 2, 128), i32),
            pltpu.VMEM((S // 128 + 2, H * 16, 128), i32),
            pltpu.VMEM((D // 2, D), i32),
            pltpu.VMEM((D, D), bf16),
            pltpu.VMEM((D, D), bf16),
            pltpu.VMEM((D, D), bf16),
            pltpu.VMEM((D, D), bf16),
            pltpu.VMEM((D, F), bf16),
            pltpu.VMEM((F, D), bf16),
            pltpu.VMEM((5, 128, 128), i32),
            pltpu.VMEM((5, 128, 128), i32),
            pltpu.VMEM((5, 128, 128), i32),
            pltpu.SMEM((1,), i32),
            pltpu.VMEM((TQ // 2, D), i32),
            pltpu.VMEM((TQ // 2, D), i32),
            pltpu.VMEM((TQ // 2, D), i32),
            pltpu.VMEM((TQ // 2, D), i32),
            pltpu.VMEM((TQ // 2, F), i32),
            pltpu.VMEM((TQ // 2, F), i32),
            pltpu.VMEM((NG, TQ // 2, 128), i32),
            pltpu.VMEM((TQ // 4, 256, 128), f32),
            pltpu.VMEM((NB, D, 128), f32),
            pltpu.VMEM((TQ, D), f32),
            pltpu.VMEM((TQ // 2, D), i32),
            pltpu.VMEM((NG, TQ // 2, 128), i32),
            pltpu.VMEM((TQ, D), f32),
            pltpu.VMEM((TQ // 2, D), i32),
            pltpu.VMEM((F,), bf16),
            pltpu.VMEM((D,), bf16),
            pltpu.SemaphoreType.DMA((9,)),
            pltpu.SemaphoreType.DMA((NU,)),
            pltpu.SemaphoreType.DMA((NU + 2,)),
        ],
        compiler_params=pltpu.CompilerParams(
            dimension_semantics=("arbitrary",),
            vmem_limit_bytes=100 * 2**20,
            disable_semaphore_checks=True),
    )(A_x, A_wqkv, A_wo, B_w1, B_b1, B_w2, B_b2)
```
